```python
import jax
import jax.numpy as jnp

def _softmax(x, axis=-1):
    return jax.nn.softmax(x, axis=axis)
def _gelu(x):
    return jax.nn.gelu(x, approximate=True)
def _silu(x):
    return jax.nn.silu(x)
def _sigmoid(x):
    return jax.nn.sigmoid(x)
def _layernorm(x, axis=-1, eps=1e-5):
    m = jnp.mean(x, axis=axis, keepdims=True)
    v = jnp.var(x, axis=axis, keepdims=True)
    return (x - m) / jnp.sqrt(v + eps)
def _scatter_add(tgt, idx, src, axis=0):
    return tgt.at[idx].add(src)
def _segment_sum(src, seg, n):
    return jax.ops.segment_sum(src, seg, n)
class _Rng:
    def __init__(self, key):
        self._k = key
    def _next(self):
        self._k, sub = jax.random.split(self._k)
        return sub
    def normal(self, shape):
        return jax.random.normal(self._next(), shape, dtype=jnp.bfloat16)
    def randint(self, lo, hi, shape):
        return jax.random.randint(self._next(), shape, lo, hi, dtype=jnp.int32)
    def uniform(self, shape, lo=0.0, hi=1.0):
        return jax.random.uniform(self._next(), shape, jnp.bfloat16, lo, hi)
    def permutation(self, n):
        return jax.random.permutation(self._next(), n)


kernel_name = 'recurrent_scan__sliding_block_cached__moe_arch_mod__decode'

def setup_inputs():
    _rng = _Rng(jax.random.key(int.from_bytes(__import__("os").urandom(4), "little")))
    _w = (lambda a: (lambda t: t.astype(jnp.bfloat16) if jnp.issubdtype(t.dtype, jnp.floating) else t)(jnp.asarray(a)))
    def _A_setup():
        B, Sq, D = 1, 1, 512
        Hq, Hkv, Sk, Dh = 32, 32, 32768, 128
        assert Hq % Hkv == 0, (Hq, Hkv)
        return {
            "x": _w((lambda *s: _rng.normal(s) * 0.05)(B, Sq, D)),
            "k_cache": _w((lambda *s: _rng.normal(s) * 0.05)(B, Hkv, Sk, Dh)),
            "v_cache": _w((lambda *s: _rng.normal(s) * 0.05)(B, Hkv, Sk, Dh)),
            "wq": _w((lambda *s: _rng.normal(s) * 0.05)(D, Hq * Dh) * (D ** -0.5)),
            "wo": _w((lambda *s: _rng.normal(s) * 0.05)(Hq * Dh, D) * ((Hq * Dh) ** -0.5)),
        }
    _A_in = _A_setup()

    def _B_setup():
        B, S, D, F, C = 1, 1, 512, 1376, 1
        return {
            "x": _w((lambda *s: _rng.normal(s) * 0.05)(B, S, D)),
            "w_r": _w((lambda *s: _rng.normal(s) * 0.05)(D)),
            "w_gate": _w((lambda *s: _rng.normal(s) * 0.05)(D, F)),
            "w_up": _w((lambda *s: _rng.normal(s) * 0.05)(D, F)),
            "w_down": _w((lambda *s: _rng.normal(s) * 0.05)(F, D)),
        }
    _B_in = _B_setup()

    return {
        "A_x": _A_in["x"],
        "A_k_cache": _A_in["k_cache"],
        "A_v_cache": _A_in["v_cache"],
        "A_wq": _A_in["wq"],
        "A_wo": _A_in["wo"],
        "B_x": _B_in["x"],
        "B_w_r": _B_in["w_r"],
        "B_w_gate": _B_in["w_gate"],
        "B_w_up": _B_in["w_up"],
        "B_w_down": _B_in["w_down"],
    }

def reference(A_x, A_k_cache, A_v_cache, A_wq, A_wo, B_x, B_w_r, B_w_gate, B_w_up, B_w_down):
    def _A_ref(x, k_cache, v_cache, wq, wo):
        B, Sq, D = x.shape
        Hq, Dh = 32, 128
        Hkv, Sk = k_cache.shape[1], k_cache.shape[2]
        W = min(4096, max(256, Sk // 4))
        rep = Hq // Hkv
        q = (lambda x, *d: x.transpose(*d))((x @ wq).reshape(B, Sq, Hq, Dh), 0, 2, 1, 3)
        k = jnp.repeat(k_cache[:, :, Sk - W:, :], rep, axis=1)
        v = jnp.repeat(v_cache[:, :, Sk - W:, :], rep, axis=1)
        scores = jnp.einsum("bhqd,bhkd->bhqk", q, k) * (Dh ** -0.5)
        p = _softmax(scores, axis=-1)
        o = jnp.einsum("bhqk,bhkd->bhqd", p, v)
        return (lambda x, *d: x.transpose(*d))(o, 0, 2, 1, 3).reshape(B, Sq, Hq * Dh) @ wo

    def _B_ref(x, w_r, w_gate, w_up, w_down):
        B, S, D = x.shape
        C = 1
        r = x @ w_r
        idx = jnp.argsort(-r, axis=-1)[:, :C]
        idx_e = jnp.repeat(idx.reshape(B, C, 1), D, axis=2)
        x_sel = jnp.take_along_axis(x, idx_e, axis=1)
        g = _silu(x_sel @ w_gate)
        u = x_sel @ w_up
        y = (g * u) @ w_down
        r_sel = _sigmoid(jnp.take_along_axis(r, idx, axis=1))
        y = y * r_sel.reshape(B, C, 1)
        b_off = (jnp.arange(B) * S).reshape(B, 1)
        flat_idx = (idx + b_off).reshape(B * C)
        zero = (x * 0.0).reshape(B * S, D)
        upd = _scatter_add(zero, flat_idx, y.reshape(B * C, D), axis=0)
        return x + upd.reshape(B, S, D)

    x = A_x
    xn = _layernorm(x, axis=-1)
    s = _A_ref(xn, A_k_cache, A_v_cache, A_wq, A_wo)
    g = _silu(_B_ref(xn, B_w_r, B_w_gate, B_w_up, B_w_down))
    return x + s * g
```

```python
import jax
import jax.numpy as jnp
from jax import lax
import jax.experimental.pallas as pl
import jax.experimental.pallas.tpu as pltpu

_NT = (((1,), (1,)), ((), ()))
_M = 8


def _make_kernel(H, SK, W, DH, D, F, NB, NWO):
    f32, bf16 = jnp.float32, jnp.bfloat16
    wo_rows = (H * DH) // NWO
    heads_per_wo = H // NWO

    def kernel(x_hbm, k_hbm, v_hbm, wq_hbm, wo_hbm, wr_hbm, wg_hbm, wu_hbm, wd_hbm,
               out_ref,
               x_v, wr_v, wq_v, wo_v, wg_v, wu_v, wd_v, k_v, v_v, q_s, o_s,
               sem_w, sem_k, sem_v, sem_wo):

        def k_copy(h, slot):
            return pltpu.make_async_copy(
                k_hbm.at[0, h, pl.ds(SK - W, W), :], k_v.at[slot], sem_k.at[slot])

        def v_copy(h, slot):
            return pltpu.make_async_copy(
                v_hbm.at[0, h, pl.ds(SK - W, W), :], v_v.at[slot], sem_v.at[slot])

        def wo_copy(c):
            return pltpu.make_async_copy(
                wo_hbm.at[pl.ds(c * wo_rows, wo_rows), :],
                wo_v.at[pl.ds(c * wo_rows, wo_rows), :], sem_wo.at[c])

        x_cp = pltpu.make_async_copy(x_hbm, x_v, sem_w.at[0])
        wr_cp = pltpu.make_async_copy(wr_hbm, wr_v, sem_w.at[1])
        wg_cp = pltpu.make_async_copy(wg_hbm, wg_v, sem_w.at[2])
        wu_cp = pltpu.make_async_copy(wu_hbm, wu_v, sem_w.at[3])
        wq_cp = pltpu.make_async_copy(wq_hbm, wq_v, sem_w.at[4])
        wd_cp = pltpu.make_async_copy(wd_hbm, wd_v, sem_w.at[5])

        x_cp.start()
        wr_cp.start()
        wg_cp.start()
        wu_cp.start()
        wq_cp.start()
        wd_cp.start()
        for h in range(NB):
            k_copy(h, h).start()
            v_copy(h, h).start()

        x_cp.wait()
        x = x_v[0].astype(f32)
        mu = jnp.mean(x, axis=-1, keepdims=True)
        xc = x - mu
        var = jnp.mean(xc * xc, axis=-1, keepdims=True)
        xn = xc / jnp.sqrt(var + 1e-5)
        xn_b = jnp.broadcast_to(xn, (_M, D)).astype(bf16)

        wr_cp.wait()
        wr = wr_v[...].astype(f32).reshape(1, D)
        r = jnp.sum(xn_b[0:1].astype(f32) * wr, axis=-1, keepdims=True)
        wg_cp.wait()
        gate = lax.dot_general(xn_b, wg_v[...], _NT, preferred_element_type=f32)
        wu_cp.wait()
        up = lax.dot_general(xn_b, wu_v[...], _NT, preferred_element_type=f32)
        hid = (gate * jax.nn.sigmoid(gate) * up).astype(bf16)

        wq_cp.wait()
        q = jnp.dot(xn_b, wq_v[...], preferred_element_type=f32).astype(bf16)
        for h in range(H):
            q_s[h] = q[:, h * DH:(h + 1) * DH]

        wd_cp.wait()
        y = jnp.dot(hid, wd_v[...], preferred_element_type=f32)[0:1]
        y = y * jax.nn.sigmoid(r)
        b = xn + (xn * 0.0 + y)
        g = b * jax.nn.sigmoid(b)

        scale = DH ** -0.5

        def head(h, carry):
            slot = h % NB
            k_copy(h, slot).wait()
            s = lax.dot_general(q_s[h], k_v[slot], _NT, preferred_element_type=f32) * scale

            @pl.when(h + NB < H)
            def _():
                k_copy(h + NB, slot).start()

            m = jnp.max(s, axis=-1, keepdims=True)
            p = jnp.exp(s - m)
            l = jnp.sum(p, axis=-1, keepdims=True)
            v_copy(h, slot).wait()
            o = jnp.dot(p.astype(bf16), v_v[slot], preferred_element_type=f32)

            @pl.when(h + NB < H)
            def _():
                v_copy(h + NB, slot).start()

            @pl.when(h + NB == H)
            def _():
                for c in range(NWO):
                    wo_copy(c).start()

            o_s[h] = (o / l).astype(bf16)
            return carry

        lax.fori_loop(0, H, head, 0)

        acc = jnp.zeros((_M, D), f32)
        for c in range(NWO):
            wo_copy(c).wait()
            for hh in range(heads_per_wo):
                h = c * heads_per_wo + hh
                acc = acc + jnp.dot(o_s[h], wo_v[pl.ds(h * DH, DH), :],
                                    preferred_element_type=f32)
        out_ref[0] = (x + acc[0:1] * g).astype(out_ref.dtype)

    return kernel


@jax.jit
def pallas_recurrent_scan__sliding_block_cached__moe_arch_mod__decode_kernel(
    A_x: jax.Array,
    A_k_cache: jax.Array,
    A_v_cache: jax.Array,
    A_wq: jax.Array,
    A_wo: jax.Array,
    B_x: jax.Array,
    B_w_r: jax.Array,
    B_w_gate: jax.Array,
    B_w_up: jax.Array,
    B_w_down: jax.Array,
):
    del B_x
    _, _, D = A_x.shape
    _, H, SK, DH = A_k_cache.shape
    F = B_w_gate.shape[1]
    W = min(4096, max(256, SK // 4))
    NB = 4
    NWO = 8
    bf16 = jnp.bfloat16

    any_spec = pl.BlockSpec(memory_space=pl.ANY)
    return pl.pallas_call(
        _make_kernel(H, SK, W, DH, D, F, NB, NWO),
        out_shape=jax.ShapeDtypeStruct(A_x.shape, A_x.dtype),
        in_specs=[any_spec] * 9,
        out_specs=pl.BlockSpec(memory_space=pltpu.VMEM),
        scratch_shapes=[
            pltpu.VMEM(A_x.shape, bf16),
            pltpu.VMEM(B_w_r.shape, bf16),
            pltpu.VMEM(A_wq.shape, bf16),
            pltpu.VMEM(A_wo.shape, bf16),
            pltpu.VMEM((F, D), bf16),
            pltpu.VMEM((F, D), bf16),
            pltpu.VMEM((F, D), bf16),
            pltpu.VMEM((NB, W, DH), bf16),
            pltpu.VMEM((NB, W, DH), bf16),
            pltpu.VMEM((H, _M, DH), bf16),
            pltpu.VMEM((H, _M, DH), bf16),
            pltpu.SemaphoreType.DMA((6,)),
            pltpu.SemaphoreType.DMA((NB,)),
            pltpu.SemaphoreType.DMA((NB,)),
            pltpu.SemaphoreType.DMA((NWO,)),
        ],
        compiler_params=pltpu.CompilerParams(vmem_limit_bytes=64 * 1024 * 1024),
    )(A_x, A_k_cache, A_v_cache, A_wq, A_wo, B_w_r, B_w_gate.T, B_w_up.T, B_w_down)
```

```python
import functools

import jax
import jax.numpy as jnp
from jax import lax
import jax.experimental.pallas as pl
import jax.experimental.pallas.tpu as pltpu

_NT = (((1,), (1,)), ((), ()))
_M = 8
_HI, _LO = 0, 1

CFG = dict(HI=0, LO=1, A_LEAD1=20, L0=3)


def _make_kernel(H, SK, W, DH, D, F, cfg):
    f32, bf16 = jnp.float32, jnp.bfloat16
    HI, LO = cfg["HI"], cfg["LO"]
    NTK = 8
    VR = W // NTK
    KA = 128
    KB = VR - KA
    KB0 = KA * NTK
    L0 = cfg["L0"]
    NBUF = 2
    scale = DH ** -0.5
    WD_LOOP = NTK * DH
    WD_REST = F - WD_LOOP
    NC = (H * DH - NTK * DH) // (2 * DH)
    A_R1, A_R0 = 32, 8

    def kernel(x_hbm, k_hbm, v_hbm, wq_hbm, wo_hbm, wr_hbm, wg_hbm, wu_hbm, wd_hbm,
               out_ref,
               x_v, wr_v, wq_v, wo_v, wg_v, wu_v, wd_v, k_v, v_v,
               qacc_s, q_s, o_s, s_s, p_s, gate_s, hid_s, g_s,
               sem_x, sem_a1, sem_a0, sem_v, sem_ka, sem_b):

        def rows_copy(src, dst, r0, n, sem):
            return pltpu.make_async_copy(src.at[pl.ds(r0, n), :], dst.at[pl.ds(r0, n), :], sem)

        def kv_copy(src, dst, h, r0, n, sem):
            return pltpu.make_async_copy(
                src.at[0, h, pl.ds(SK - W + r0, n), :], dst.at[h % NBUF, pl.ds(r0, n), :], sem)

        def static(p):
            return isinstance(p, int)

        def p1_copies(p, j):
            if static(p) and p >= H:
                i = (p - H) * NTK + j
                if i >= NC:
                    return []
                return [rows_copy(wo_hbm, wo_v, NTK * DH + 2 * DH * i, 160, sem_v.at[j])]
            if static(p) and p < 0:
                a = rows_copy(wd_hbm, wd_v, DH * j, DH, sem_v.at[j])
            else:
                a = kv_copy(v_hbm, v_v, p, VR * j, VR, sem_v.at[j])
            if static(p) and p == H - 1:
                b = rows_copy(wo_hbm, wo_v, DH * j, 32, sem_ka.at[j])
            else:
                b = kv_copy(k_hbm, k_v, p + 1, KA * j, KA, sem_ka.at[j])
            return [a, b]

        def p0_copy(p, j, part):
            if static(p) and p >= H - 1:
                if p == H - 1:
                    r0 = DH * j + 32
                else:
                    i = (p - H) * NTK + j
                    if i >= NC:
                        return None
                    r0 = NTK * DH + 2 * DH * i + 160
                if part is None:
                    return rows_copy(wo_hbm, wo_v, r0, 96, sem_b.at[j])
                return rows_copy(wo_hbm, wo_v, r0 + 48 * part, 48, sem_b.at[j])
            r0 = KB0 + KB * j
            if part is None:
                return kv_copy(k_hbm, k_v, p + 1, r0, KB, sem_b.at[j])
            return kv_copy(k_hbm, k_v, p + 1, r0 + (KB // 2) * part, KB // 2, sem_b.at[j])

        def ahead(p, j, n):
            return p + (j + n) // NTK, (j + n) % NTK

        def tick(p, j, compute):
            for c in p1_copies(p, j):
                c.wait()
            c = p0_copy(*ahead(p, j, L0), 0)
            if c is not None:
                c.start(priority=HI)
            res = compute()
            for c in p1_copies(p + 1, j):
                c.start(priority=LO)
            c = p0_copy(*ahead(p, j, 1), None)
            if c is not None:
                c.wait()
            c = p0_copy(*ahead(p, j, L0), 1)
            if c is not None:
                c.start(priority=HI)
            return res

        def qk_piece(h, j, m_run):
            slot = h % NBUF
            kk = jnp.concatenate([k_v[slot, pl.ds(KA * j, KA), :],
                                  k_v[slot, pl.ds(KB0 + KB * j, KB), :]], axis=0)
            s = lax.dot_general(q_s[h], kk, _NT, preferred_element_type=f32)
            s_s[:, pl.ds(KA * j, KA)] = s[:, :KA]
            s_s[:, pl.ds(KB0 + KB * j, KB)] = s[:, KA:]
            for t in range(VR // 128):
                st = s[:, t * 128:(t + 1) * 128]
                m_run = st if m_run is None else jnp.maximum(m_run, st)
            return m_run

        def softmax_num(m_run):
            m = jnp.max(m_run, axis=-1, keepdims=True)
            p = jnp.exp((s_s[...] - m) * scale)
            p_s[...] = p.astype(bf16)
            parts = [p[:, t * 128:(t + 1) * 128] for t in range(W // 128)]
            while len(parts) > 1:
                parts = [a + b for a, b in zip(parts[0::2], parts[1::2])]
            return parts[0]

        def pv_piece(h, j, acc):
            o = jnp.dot(p_s[:, pl.ds(VR * j, VR)], v_v[h % NBUF, pl.ds(VR * j, VR), :],
                        preferred_element_type=f32)
            return o if acc is None else acc + o

        def wo_slab(h):
            return jnp.dot(o_s[h], wo_v[pl.ds(h * DH, DH), :], preferred_element_type=f32)

        n_wq = D // 8
        n_wg = F // 32
        wu_split = (n_wq - n_wg) * 32
        n_tail = (F - wu_split) // 64
        assert n_tail * 64 == F - wu_split and n_tail * 32 == WD_REST
        NA = n_wq + n_tail

        def a1_copy(a):
            sem = sem_a1.at[a % A_R1]
            if a < n_wq:
                return rows_copy(wq_hbm, wq_v, 8 * a, 8, sem)
            return rows_copy(wu_hbm, wu_v, wu_split + 64 * (a - n_wq), 64, sem)

        def a0_copy(a):
            sem = sem_a0.at[a % A_R0]
            if a < n_wg:
                return rows_copy(wg_hbm, wg_v, 32 * a, 32, sem)
            if a < n_wq:
                return rows_copy(wu_hbm, wu_v, 32 * (a - n_wg), 32, sem)
            return rows_copy(wd_hbm, wd_v, WD_LOOP + 32 * (a - n_wq), 32, sem)

        A_LEAD1 = cfg["A_LEAD1"]
        N0 = 2 * L0
        assert A_LEAD1 <= A_R1 and N0 <= A_R0
        p0_fifo = [functools.partial(a0_copy, a) for a in range(NA)]
        p0_fifo += [functools.partial(p0_copy, -1, j, part) for j in range(L0) for part in (0, 1)]

        x_cp = pltpu.make_async_copy(x_hbm, x_v, sem_x.at[0])
        wr_cp = pltpu.make_async_copy(wr_hbm, wr_v, sem_x.at[1])
        a1_copy(0).start(priority=LO)
        x_cp.start(priority=HI)
        wr_cp.start(priority=HI)
        for a in range(max(A_LEAD1, N0)):
            if a < N0:
                p0_fifo[a]().start(priority=HI)
            if 1 <= a < A_LEAD1:
                a1_copy(a).start(priority=LO)

        x_cp.wait()
        wr_cp.wait()
        x = x_v[0].astype(f32)
        mu = jnp.mean(x, axis=-1, keepdims=True)
        xc = x - mu
        var = jnp.mean(xc * xc, axis=-1, keepdims=True)
        xn = xc / jnp.sqrt(var + 1e-5)
        xn_b = jnp.broadcast_to(xn, (_M, D)).astype(bf16)
        wr = wr_v[...].astype(f32).reshape(1, D)
        r_gate = jax.nn.sigmoid(jnp.sum(xn * wr, axis=-1, keepdims=True))

        def q_slab(k, half):
            cols = pl.ds(half * (H * DH // 2), H * DH // 2)
            part = jnp.dot(xn_b[:, k * 128:(k + 1) * 128], wq_v[pl.ds(k * 128, 128), cols],
                           preferred_element_type=f32)
            if k > 0:
                part = part + qacc_s[:, cols]
            if k < D // 128 - 1:
                qacc_s[:, cols] = part
            else:
                qb = part.astype(bf16)
                for hh in range(H // 2):
                    q_s[half * (H // 2) + hh] = qb[:, hh * DH:(hh + 1) * DH]

        def gate_piece(c0, n):
            gate_s[:, pl.ds(c0, n)] = lax.dot_general(
                xn_b, wg_v[pl.ds(c0, n), :], _NT, preferred_element_type=f32)

        def up_piece(c0, n):
            up = lax.dot_general(xn_b, wu_v[pl.ds(c0, n), :], _NT, preferred_element_type=f32)
            gate = gate_s[:, pl.ds(c0, n)]
            hid_s[:, pl.ds(c0, n)] = (gate * jax.nn.sigmoid(gate) * up).astype(bf16)

        jobs = {}

        def add_job(a, fn):
            while a in jobs and a < NA - 1:
                a += 1
            jobs.setdefault(a, []).append(fn)

        for k in range(D // 128):
            for half in range(2):
                add_job(16 * k + 15, functools.partial(q_slab, k, half))
        for c0 in range(0, F, 256):
            n = min(256, F - c0)
            add_job((c0 + n) // 32 - 1, functools.partial(gate_piece, c0, n))
        for c0 in range(0, F, 256):
            n = min(256, F - c0)
            end = c0 + n
            if end <= wu_split:
                a = n_wg + end // 32 - 1
            else:
                a = n_wq + -(-(end - wu_split) // 64) - 1
            add_job(a, functools.partial(up_piece, c0, n))

        first = NA - A_LEAD1
        b_start = {first + (j * A_LEAD1) // NTK: j for j in range(NTK)}
        for a in range(NA):
            a1_copy(a).wait()
            a0_copy(a).wait()
            p0_fifo[a + N0]().start(priority=HI)
            if a + A_LEAD1 < NA:
                a1_copy(a + A_LEAD1).start(priority=LO)
            if a in b_start:
                for c in p1_copies(-1, b_start[a]):
                    c.start(priority=LO)
            for fn in jobs.get(a, []):
                fn()
        p0_copy(-1, 0, None).wait()

        m_run = None
        y = None
        for j in range(NTK):
            def comp(j=j, m_run=m_run, y=y):
                m_new = qk_piece(0, j, m_run)
                part = jnp.dot(hid_s[:, pl.ds(DH * j, DH)], wd_v[pl.ds(DH * j, DH), :],
                               preferred_element_type=f32)
                if j == 0:
                    part = part + jnp.dot(hid_s[:, pl.ds(WD_LOOP, WD_REST)],
                                          wd_v[pl.ds(WD_LOOP, WD_REST), :],
                                          preferred_element_type=f32)
                y_new = part if y is None else y + part
                if j == NTK - 1:
                    b = xn + (xn * 0.0 + y_new[0:1] * r_gate)
                    g_s[...] = b * jax.nn.sigmoid(b)
                    m_new = softmax_num(m_new)
                return m_new, y_new
            m_run, y = tick(-1, j, comp)
        l_vec = m_run

        def period(h, l_vec):
            m_run = None
            acc = None
            for j in range(NTK):
                def comp(j=j, m_run=m_run, acc=acc):
                    acc_new = pv_piece(h, j, acc)
                    m_new = qk_piece(h + 1, j, m_run)
                    if j == NTK - 1:
                        l = jnp.sum(l_vec, axis=-1, keepdims=True)
                        o_s[h] = (acc_new / l).astype(bf16)
                        m_new = softmax_num(m_new)
                    return m_new, acc_new
                m_run, acc = tick(h, j, comp)
            return m_run

        l_vec = lax.fori_loop(0, H - 2, period, l_vec)
        l_vec = period(H - 2, l_vec)

        acc = None
        out = None
        for j in range(NTK):
            def comp(j=j, acc=acc, out=out):
                acc_new = pv_piece(H - 1, j, acc)
                part = wo_slab(j)
                if j == NTK - 1:
                    l = jnp.sum(l_vec, axis=-1, keepdims=True)
                    o_s[H - 1] = (acc_new / l).astype(bf16)
                return acc_new, (part if out is None else out + part)
            acc, out = tick(H - 1, j, comp)

        for i in range(NC):
            def comp(i=i, out=out):
                return out + wo_slab(NTK + 2 * i) + wo_slab(NTK + 2 * i + 1)
            out = tick(H + i // NTK, i % NTK, comp)
        out_ref[0] = (x_v[0].astype(f32) + out[0:1] * g_s[...]).astype(out_ref.dtype)

    scratch = [
        pltpu.VMEM((1, 1, D), bf16),
        pltpu.VMEM((D,), bf16),
        pltpu.VMEM((D, H * DH), bf16),
        pltpu.VMEM((H * DH, D), bf16),
        pltpu.VMEM((F, D), bf16),
        pltpu.VMEM((F, D), bf16),
        pltpu.VMEM((F, D), bf16),
        pltpu.VMEM((NBUF, W, DH), bf16),
        pltpu.VMEM((NBUF, W, DH), bf16),
        pltpu.VMEM((_M, H * DH), f32),
        pltpu.VMEM((H, _M, DH), bf16),
        pltpu.VMEM((H, _M, DH), bf16),
        pltpu.VMEM((_M, W), f32),
        pltpu.VMEM((_M, W), bf16),
        pltpu.VMEM((_M, F), f32),
        pltpu.VMEM((_M, F), bf16),
        pltpu.VMEM((1, D), f32),
        pltpu.SemaphoreType.DMA((2,)),
        pltpu.SemaphoreType.DMA((A_R1,)),
        pltpu.SemaphoreType.DMA((A_R0,)),
        pltpu.SemaphoreType.DMA((NTK,)),
        pltpu.SemaphoreType.DMA((NTK,)),
        pltpu.SemaphoreType.DMA((NTK,)),
    ]
    return kernel, scratch


@jax.jit
def pallas_recurrent_scan__sliding_block_cached__moe_arch_mod__decode_kernel(
    A_x: jax.Array,
    A_k_cache: jax.Array,
    A_v_cache: jax.Array,
    A_wq: jax.Array,
    A_wo: jax.Array,
    B_x: jax.Array,
    B_w_r: jax.Array,
    B_w_gate: jax.Array,
    B_w_up: jax.Array,
    B_w_down: jax.Array,
):
    del B_x
    _, _, D = A_x.shape
    _, H, SK, DH = A_k_cache.shape
    F = B_w_gate.shape[1]
    W = min(4096, max(256, SK // 4))
    kernel, scratch = _make_kernel(H, SK, W, DH, D, F, CFG)
    any_spec = pl.BlockSpec(memory_space=pl.ANY)
    return pl.pallas_call(
        kernel,
        out_shape=jax.ShapeDtypeStruct(A_x.shape, A_x.dtype),
        in_specs=[any_spec] * 9,
        out_specs=pl.BlockSpec(memory_space=pltpu.VMEM),
        scratch_shapes=scratch,
        compiler_params=pltpu.CompilerParams(
            vmem_limit_bytes=48 * 1024 * 1024,
            disable_bounds_checks=True,
            disable_semaphore_checks=True),
    )(A_x, A_k_cache, A_v_cache, A_wq, A_wo, B_w_r, B_w_gate.T, B_w_up.T, B_w_down)
```

```python
import functools

import jax
import jax.numpy as jnp
from jax import lax
import jax.experimental.pallas as pl
import jax.experimental.pallas.tpu as pltpu

_NT = (((1,), (1,)), ((), ()))
_M = 8

CFG = dict(HI=0, LO=1, N0=18, G_KV=14, G_WQ=14, G_WO=14, G_WG=0, G_WU=16, G_WD=0,
           KSUB=4, VSUB=2, JOBGAP=3)

_BT = 32
_BB = 2


def _rects(name, t0, t1, ct):
    out = []
    while t0 < t1:
        r, c = divmod(t0, ct)
        if c or t1 - t0 < ct:
            n = min(ct - c, t1 - t0)
            out.append((name, 8 * r, 8, 128 * c, 128 * n))
            t0 += n
        else:
            rows = (t1 - t0) // ct
            out.append((name, 8 * r, 8 * rows, 0, 128 * ct))
            t0 += rows * ct
    return out


def _weight_blocks(name, rows, cols, g):
    ct = cols // 128
    total = rows // 8 * ct
    cuts = sorted({0, total} | set(range(g % _BT, total, _BT)))
    out = []
    for lo, hi in zip(cuts[:-1], cuts[1:]):
        (burst,) = _rects(name, hi - _BB, hi, ct)
        out.append((_rects(name, lo, hi - _BB, ct), burst))
    return out


def _tiles(piece):
    name, r0, nr, c0, nc = piece
    return {(name, r, c) for r in range(r0 // 8, (r0 + nr) // 8) for c in range(c0 // 128, (c0 + nc) // 128)}


def _interleave(a, b):
    out = []
    for i in range(max(len(a), len(b))):
        out += a[i:i + 1] + b[i:i + 1]
    return out


def _make_kernel(H, SK, W, DH, D, F, cfg):
    f32, bf16 = jnp.float32, jnp.bfloat16
    HI, LO, N0 = cfg["HI"], cfg["LO"], cfg["N0"]
    BR = _BT * 8
    G0 = cfg["G_KV"] * 8
    NBLK = (W - G0) // BR
    NS = 2 * NBLK
    NBUF = 2
    scale = DH ** -0.5

    tail0 = G0 + NBLK * BR
    n_head = max(1, round(NBLK * G0 / (G0 + W - tail0)))

    def cut(lo, hi, k):
        b = [lo + (hi - lo) // 8 * i // k * 8 for i in range(k + 1)]
        return [(x, y - x) for x, y in zip(b[:-1], b[1:])]
    frag_head, frag_tail = cut(0, G0, n_head), cut(tail0, W, NBLK - n_head)

    def kv_blocks(name, h):
        return [[(name, h, G0 + BR * b, BR)] for b in range(NBLK)]

    def kv_bursts(name, h):
        return [(name, h, r, n) for r, n in frag_head + frag_tail]

    def set_slot(p, j):
        return [("V", p, G0 + BR * (j // 2), BR)] if j % 2 == 0 else [("K", p + 1, G0 + BR * (j // 2), BR)]

    set_burst_list = ([("V", r, n) for r, n in frag_head] + [("K", r, n) for r, n in frag_head]
                      + [("V", r, n) for r, n in frag_tail] + [("K", r, n) for r, n in frag_tail])

    def set_burst(p, j):
        name, r, n = set_burst_list[j]
        return (name, p if name == "V" else p + 1, r, n)

    wq_b = _weight_blocks("wq", D, H * DH, cfg["G_WQ"])
    wg_b = _weight_blocks("wg", F, D, cfg["G_WG"])
    wu_b = _weight_blocks("wu", F, D, cfg["G_WU"])
    wd_b = _weight_blocks("wd", F, D, cfg["G_WD"])
    wo_b = _weight_blocks("wo", H * DH, D, cfg["G_WO"])
    k0_b = list(zip(kv_blocks("K", 0), kv_bursts("K", 0)))
    n_all = len(wq_b) + len(wg_b) + len(wu_b) + len(wd_b) + len(k0_b)
    move = (n_all + 1) // 2 - len(wq_b)
    pro = _interleave(wq_b + wd_b[len(wd_b) - move:], wg_b + wu_b + wd_b[:len(wd_b) - move] + k0_b)
    NP = len(pro)
    rest = wo_b[NBLK:]
    half = (len(rest) + 1) // 2
    wo_order = wo_b[:NBLK] + _interleave(rest[:half], rest[half:])
    epi_slots = (_interleave(kv_blocks("V", H - 1), [b for b, _ in wo_order[:NBLK]])
                 + [b for b, _ in wo_order[NBLK:]])
    epi_bursts = kv_bursts("V", H - 1) + [s for _, s in wo_order]
    NE = len(epi_slots)
    E0 = NP + NS * (H - 1)

    def kernel(x_hbm, k_hbm, v_hbm, wq_hbm, wo_hbm, wr_hbm, wg_hbm, wu_hbm, wd_hbm,
               out_ref,
               x_v, wr_v, wq_v, wo_v, wg_v, wu_v, wd_v, kv_v,
               qacc_s, q_s, o_s, s_s, p_s, gate_s, hid_s, g_s,
               sem_x, sem1, sem0):
        mats = dict(wq=(wq_hbm, wq_v), wo=(wo_hbm, wo_v), wg=(wg_hbm, wg_v), wu=(wu_hbm, wu_v),
                    wd=(wd_hbm, wd_v))

        def buf(name, h):
            return (h & (NBUF - 1)) + (NBUF if name == "V" else 0)

        def copy(piece, sem):
            if piece[0] in mats:
                name, r0, nr, c0, nc = piece
                src, dst = mats[name]
                return pltpu.make_async_copy(src.at[pl.ds(r0, nr), pl.ds(c0, nc)],
                                             dst.at[pl.ds(r0, nr), pl.ds(c0, nc)], sem)
            name, h, r0, nr = piece
            src = k_hbm if name == "K" else v_hbm
            return pltpu.make_async_copy(src.at[0, h, pl.ds(SK - W + r0, nr), :],
                                         kv_v.at[buf(name, h), pl.ds(r0, nr), :], sem)

        def locate(p, j):
            if p is None or isinstance(p, int):
                return None, j if p is None else NP + NS * p + j
            return (p + j // NS, j % NS), NP + j

        def slot_pieces(p, j):
            dyn, gi = locate(p, j)
            if dyn is not None:
                return set_slot(*dyn), gi
            if gi < NP:
                return pro[gi][0], gi
            if gi < E0:
                return set_slot(*divmod(gi - NP, NS)), gi
            return (epi_slots[gi - E0] if gi - E0 < NE else []), gi

        def burst_pieces(p, j):
            dyn, gi = locate(p, j)
            if dyn is not None:
                return [set_burst(*dyn)], gi
            if gi < NP:
                return [pro[gi][1]], gi
            if gi < E0:
                return [set_burst(*divmod(gi - NP, NS))], gi
            return epi_bursts[gi - E0:gi - E0 + 1], gi

        landed = set()

        def start_slot(p, j):
            pieces, gi = slot_pieces(p, j)
            for pc in pieces:
                copy(pc, sem1.at[gi % NS]).start(priority=LO)

        def start_burst(p, j):
            pieces, gi = burst_pieces(p, j)
            for pc in pieces:
                copy(pc, sem0.at[gi % NS]).start(priority=HI)

        def wait_both(p, j):
            for (pieces, gi), sem in ((slot_pieces(p, j), sem1), (burst_pieces(p, j), sem0)):
                for pc in pieces:
                    copy(pc, sem.at[gi % NS]).wait()
                    if pc[0] in mats:
                        landed.update(_tiles(pc))

        class Jobs:
            def __init__(self):
                self.todo, self.done, self.cool = [], set(), 0

            def add(self, key, need, after, fn):
                self.todo.append((key, _tiles(need), set(after), fn))

            def ready(self):
                return [j for j in self.todo if j[1] <= landed and j[2] <= self.done]

            def run(self, job):
                self.todo.remove(job)
                if not cfg.get("NOJOBS") or job[0] == 0:
                    job[3]()
                self.done.add(job[0])

            def step(self, gap, n=1):
                self.cool -= 1
                ready = self.ready()
                if self.cool <= 0 and len(ready) >= min(n, len(self.todo)) and ready:
                    for job in ready[:n]:
                        self.run(job)
                    self.cool = gap

            def flush(self):
                while self.todo:
                    self.run(self.ready()[0])

        x_cp = pltpu.make_async_copy(x_hbm, x_v, sem_x.at[0])
        wr_cp = pltpu.make_async_copy(wr_hbm, wr_v, sem_x.at[1])
        start_slot(None, 0)
        x_cp.start(priority=HI)
        wr_cp.start(priority=HI)
        for i in range(NS):
            if i > 0:
                start_slot(None, i)
            if i < N0:
                start_burst(None, i)

        x_cp.wait()
        wr_cp.wait()
        x = x_v[0].astype(f32)
        mu = jnp.mean(x, axis=-1, keepdims=True)
        xc = x - mu
        var = jnp.mean(xc * xc, axis=-1, keepdims=True)
        xn = xc / jnp.sqrt(var + 1e-5)
        xn_b = jnp.broadcast_to(xn, (_M, D)).astype(bf16)
        wr = wr_v[...].astype(f32).reshape(1, D)
        r_gate = jax.nn.sigmoid(jnp.sum(xn * wr, axis=-1, keepdims=True))

        QH = H * DH // 2

        def q_slab(k, half):
            cols = pl.ds(half * QH, QH)
            part = jnp.dot(xn_b[:, k * 128:(k + 1) * 128], wq_v[pl.ds(k * 128, 128), cols],
                           preferred_element_type=f32)
            if k > 0:
                part = part + qacc_s[:, cols]
            if k < D // 128 - 1:
                qacc_s[:, cols] = part
            else:
                qb = part.astype(bf16)
                for hh in range(H // 2):
                    q_s[half * (H // 2) + hh] = qb[:, hh * DH:(hh + 1) * DH]

        def gate_piece(c0, n):
            gate_s[:, pl.ds(c0, n)] = lax.dot_general(
                xn_b, wg_v[pl.ds(c0, n), :], _NT, preferred_element_type=f32)

        def up_piece(c0, n):
            up = lax.dot_general(xn_b, wu_v[pl.ds(c0, n), :], _NT, preferred_element_type=f32)
            gate = gate_s[:, pl.ds(c0, n)]
            hid_s[:, pl.ds(c0, n)] = (gate * jax.nn.sigmoid(gate) * up).astype(bf16)

        def down_piece(c0, n):
            y = jnp.dot(hid_s[:, pl.ds(c0, n)], wd_v[pl.ds(c0, n), :],
                        preferred_element_type=f32)[0:1]
            if c0 > 0:
                y = y + g_s[...]
            if c0 + n == F:
                b = xn + (xn * 0.0 + y * r_gate)
                y = b * jax.nn.sigmoid(b)
            g_s[...] = y

        jobs = Jobs()
        for k in range(D // 128):
            for half in range(2):
                jobs.add(("q", k, half), ("wq", 128 * k, 128, half * QH, QH),
                         [("q", k - 1, half)] if k else [], functools.partial(q_slab, k, half))
        for c0 in range(0, F, 256):
            n = min(256, F - c0)
            jobs.add(("g", c0), ("wg", c0, n, 0, D), [], functools.partial(gate_piece, c0, n))
            jobs.add(("u", c0), ("wu", c0, n, 0, D), [("g", c0)], functools.partial(up_piece, c0, n))
        for c0 in range(0, F, 512):
            n = min(512, F - c0)
            after = [("u", c) for c in range(c0, c0 + n, 256)] + ([("d", c0 - 512)] if c0 else [])
            jobs.add(("d", c0), ("wd", c0, n, 0, D), after, functools.partial(down_piece, c0, n))

        for i in range(NP):
            wait_both(None, i)
            start_burst(None, i + N0)
            start_slot(None, i + NS)
            if i < NP - 1:
                jobs.step(cfg["JOBGAP"])

        def qk(h, anchor):
            m_run = None
            rows = W // cfg["KSUB"]
            for c in range(cfg["KSUB"]):
                s = lax.dot_general(q_s[h], kv_v[buf("K", h), pl.ds(c * rows, rows), :], _NT,
                                    preferred_element_type=f32)
                anchor()
                s_s[:, pl.ds(c * rows, rows)] = s
                for t in range(rows // 128):
                    st = s[:, t * 128:(t + 1) * 128]
                    m_run = st if m_run is None else jnp.maximum(m_run, st)
            return m_run

        def softmax_num(m_run):
            m = jnp.max(m_run, axis=-1, keepdims=True)
            p = jnp.exp((s_s[...] - m) * scale)
            p_s[...] = p.astype(bf16)
            parts = [p[:, t * 128:(t + 1) * 128] for t in range(W // 128)]
            while len(parts) > 1:
                parts = [a + b for a, b in zip(parts[0::2], parts[1::2])]
            return parts[0]

        def pv(h, l_vec, anchor):
            acc = None
            rows = W // cfg["VSUB"]
            for c in range(cfg["VSUB"]):
                o = jnp.dot(p_s[:, pl.ds(c * rows, rows)],
                            kv_v[buf("V", h), pl.ds(c * rows, rows), :], preferred_element_type=f32)
                anchor()
                acc = o if acc is None else o + acc
            l = jnp.sum(l_vec, axis=-1, keepdims=True)
            o_s[h] = (acc / l).astype(bf16)

        def period(p, l_vec, extra=None, per_slot=None):
            issued = [0]

            def anchor():
                start_burst(p, issued[0] + N0)
                issued[0] += 1

            if extra is not None:
                extra()
            if cfg.get("NOATT"):
                l_new = jnp.zeros((_M, 128), f32)
            else:
                m_run = qk(p, anchor)
                if l_vec is not None:
                    pv(p - 1, l_vec, anchor)
                l_new = softmax_num(m_run)
            skip = issued[0]
            for j in range(NS):
                wait_both(p, j)
                if j == 0 or j > skip:
                    anchor()
                start_slot(p, j + NS)
                if per_slot is not None and j > skip:
                    per_slot()
            return l_new

        l_vec = period(0, None, extra=jobs.flush)
        l_vec = lax.fori_loop(1, H - 2, period, l_vec)
        l_vec = period(H - 2, l_vec)

        out = [None]

        def wo_slab(h):
            part = jnp.dot(o_s[h], wo_v[pl.ds(h * DH, DH), :], preferred_element_type=f32)
            out[0] = part if out[0] is None else part + out[0]

        ojobs = Jobs()
        for h in range(H):
            ojobs.add(h, ("wo", h * DH, DH, 0, D), ["pv"] if h == H - 1 else [],
                      functools.partial(wo_slab, h))
        l_vec = period(H - 1, l_vec, per_slot=lambda: ojobs.step(2, 2))
        if not cfg.get("NOATT"):
            pv(H - 1, l_vec, lambda: None)
        ojobs.done.add("pv")
        for j in range(NE - NS):
            wait_both(H, j)
            start_burst(H, j + N0)
            start_slot(H, j + NS)
            ojobs.step(2, 2 if j < NE - NS - 4 else 1)
        ojobs.flush()
        out_ref[0] = (x_v[0].astype(f32) + out[0][0:1] * g_s[...]).astype(out_ref.dtype)

    scratch = [
        pltpu.VMEM((1, 1, D), bf16),
        pltpu.VMEM((D,), bf16),
        pltpu.VMEM((D, H * DH), bf16),
        pltpu.VMEM((H * DH, D), bf16),
        pltpu.VMEM((F, D), bf16),
        pltpu.VMEM((F, D), bf16),
        pltpu.VMEM((F, D), bf16),
        pltpu.VMEM((2 * NBUF, W, DH), bf16),
        pltpu.VMEM((_M, H * DH), f32),
        pltpu.VMEM((H, _M, DH), bf16),
        pltpu.VMEM((H, _M, DH), bf16),
        pltpu.VMEM((_M, W), f32),
        pltpu.VMEM((_M, W), bf16),
        pltpu.VMEM((_M, F), f32),
        pltpu.VMEM((_M, F), bf16),
        pltpu.VMEM((1, D), f32),
        pltpu.SemaphoreType.DMA((2,)),
        pltpu.SemaphoreType.DMA((NS,)),
        pltpu.SemaphoreType.DMA((NS,)),
    ]
    return kernel, scratch


@jax.jit
def pallas_recurrent_scan__sliding_block_cached__moe_arch_mod__decode_kernel(
    A_x: jax.Array,
    A_k_cache: jax.Array,
    A_v_cache: jax.Array,
    A_wq: jax.Array,
    A_wo: jax.Array,
    B_x: jax.Array,
    B_w_r: jax.Array,
    B_w_gate: jax.Array,
    B_w_up: jax.Array,
    B_w_down: jax.Array,
):
    del B_x
    _, _, D = A_x.shape
    _, H, SK, DH = A_k_cache.shape
    F = B_w_gate.shape[1]
    W = min(4096, max(256, SK // 4))
    kernel, scratch = _make_kernel(H, SK, W, DH, D, F, CFG)
    any_spec = pl.BlockSpec(memory_space=pl.ANY)
    return pl.pallas_call(
        kernel,
        out_shape=jax.ShapeDtypeStruct(A_x.shape, A_x.dtype),
        in_specs=[any_spec] * 9,
        out_specs=pl.BlockSpec(memory_space=pltpu.VMEM),
        scratch_shapes=scratch,
        compiler_params=pltpu.CompilerParams(
            vmem_limit_bytes=48 * 1024 * 1024,
            disable_bounds_checks=True,
            disable_semaphore_checks=True),
    )(A_x, A_k_cache, A_v_cache, A_wq, A_wo, B_w_r, B_w_gate.T, B_w_up.T, B_w_down)
```

```python
import functools

import jax
import jax.numpy as jnp
from jax import lax
import jax.experimental.pallas as pl
import jax.experimental.pallas.tpu as pltpu

_NT = (((1,), (1,)), ((), ()))
_M = 8

CFG = dict(HI=0, LO=1, N0=14, G_KV=14, G_WQ=14, G_WO=12, G_WG=0, G_WU=16, G_WD=0,
           KSUB=4, VSUB=2, JOBGAP=3, WO_STREAMS=4, R_PRO=2, R_WO=6)

_BT = 32


def _rects(name, t0, t1, ct):
    out = []
    while t0 < t1:
        r, c = divmod(t0, ct)
        if c or t1 - t0 < ct:
            n = min(ct - c, t1 - t0)
            out.append((name, 8 * r, 8, 128 * c, 128 * n))
            t0 += n
        else:
            rows = (t1 - t0) // ct
            out.append((name, 8 * r, 8 * rows, 0, 128 * ct))
            t0 += rows * ct
    return out


def _split_weight(name, rows, cols, g, reserve):
    ct = cols // 128
    total = rows // 8 * ct
    lo = g % _BT + reserve * _BT
    hi = lo + (total - lo) // _BT * _BT
    blocks = [_rects(name, t, t + _BT, ct) for t in range(lo, hi, _BT)]
    small = [(name, t, ct) for t in list(range(0, lo, 2)) + list(range(hi, total, 2))]
    return blocks, small


def _fit(small, n):
    out, extra, i = [], len(small) - n, 0
    while i < len(small):
        name, t, ct = small[i]
        if extra > 0 and t % 4 == 0 and small[i + 1:i + 2] == [(name, t + 2, ct)] and i % 4 == 0:
            out.append(_rects(name, t, t + 4, ct))
            i, extra = i + 2, extra - 1
        else:
            out.append(_rects(name, t, t + 2, ct))
            i += 1
    assert extra <= 0
    return out + [[]] * (n - len(out))


def _tiles(piece):
    name, r0, nr, c0, nc = piece
    return {(name, r, c) for r in range(r0 // 8, (r0 + nr) // 8) for c in range(c0 // 128, (c0 + nc) // 128)}


def _rotate(*streams):
    out = []
    for i in range(max(len(s) for s in streams)):
        for s in streams:
            out += s[i:i + 1]
    return out


def _make_kernel(H, SK, W, DH, D, F, cfg):
    f32, bf16 = jnp.float32, jnp.bfloat16
    HI, LO, N0 = cfg["HI"], cfg["LO"], cfg["N0"]
    BR = _BT * 8
    G0 = cfg["G_KV"] * 8
    NBLK = (W - G0) // BR
    NS = 2 * NBLK
    scale = DH ** -0.5
    hb = (NBLK + 1) // 2
    border = _rotate(list(range(hb)), list(range(hb, NBLK)))

    tail0 = G0 + NBLK * BR
    n_head = max(1, round(NBLK * G0 / (G0 + W - tail0)))

    def cut(lo, hi, k):
        b = [lo + (hi - lo) // 8 * i // k * 8 for i in range(k + 1)]
        return [(x, y - x) for x, y in zip(b[:-1], b[1:])]
    frag_head, frag_tail = cut(0, G0, n_head), cut(tail0, W, NBLK - n_head)
    frags = ([("V", r, n) for r, n in frag_head] + [("K", r, n) for r, n in frag_head]
             + [("V", r, n) for r, n in frag_tail] + [("K", r, n) for r, n in frag_tail])

    def kv_slot(t, j):
        b0, b1 = border[j // 4], border[(NS + j) // 4]
        row = G0 + BR * b0 + (t & 1) * (BR * (b1 - b0))
        if not isinstance(row, int):
            row = pl.multiple_of(row, 8)
        return [("VK"[j % 2], t ^ ((j % 4) // 2), row, BR)]

    def kv_burst(t, j):
        name, r, n = frags[j]
        return [(name, t + 2, r, n)]

    wq_b, wq_s = _split_weight("wq", D, H * DH, cfg["G_WQ"], cfg["R_PRO"])
    wg_b, wg_s = _split_weight("wg", F, D, cfg["G_WG"], 0)
    wu_b, wu_s = _split_weight("wu", F, D, cfg["G_WU"], 0)
    wd_b, wd_s = _split_weight("wd", F, D, cfg["G_WD"], 0)
    hq, hd = (len(wq_b) + 1) // 2, (len(wd_b) + 1) // 2
    pro_slots = _rotate(wg_b + wd_b[:hd], wq_b[:hq], wu_b + wd_b[hd:], wq_b[hq:])
    NP = len(pro_slots)
    pro_bursts = (_fit(wu_s + wq_s + wg_s + wd_s, NP - 2 * NS)
                  + [kv_burst(t, j) for t in (-2, -1) for j in range(NS)])
    wo_b, wo_s = _split_weight("wo", H * DH, D, cfg["G_WO"], cfg["R_WO"])
    ns = cfg["WO_STREAMS"]
    cuts = [len(wo_b) * i // ns for i in range(ns + 1)]
    epi_slots = _rotate(*[wo_b[a:b][::-1] for a, b in zip(cuts[:-1], cuts[1:])][::-1])[::-1]
    NE = len(epi_slots)
    epi_bursts = _fit(wo_s, 2 * NS + NE)
    E1 = NP + NS * H
    E0 = NP + NS * (H - 2)

    def kernel(x_hbm, k_hbm, v_hbm, wq_hbm, wo_hbm, wr_hbm, wg_hbm, wu_hbm, wd_hbm,
               out_ref,
               x_v, wr_v, wq_v, wo_v, wg_v, wu_v, wd_v, kv_v,
               qacc_s, q_s, o_s, s_s, p_s, gate_s, hid_s, g_s,
               sem_x, sem1, sem0):
        mats = dict(wq=(wq_hbm, wq_v), wo=(wo_hbm, wo_v), wg=(wg_hbm, wg_v), wu=(wu_hbm, wu_v),
                    wd=(wd_hbm, wd_v))

        def buf(name, h):
            return h + (H if name == "V" else 0)

        def copy(piece, sem):
            if piece[0] in mats:
                name, r0, nr, c0, nc = piece
                src, dst = mats[name]
                return pltpu.make_async_copy(src.at[pl.ds(r0, nr), pl.ds(c0, nc)],
                                             dst.at[pl.ds(r0, nr), pl.ds(c0, nc)], sem)
            name, h, r0, nr = piece
            src = k_hbm if name == "K" else v_hbm
            rs = SK - W + r0
            if not isinstance(rs, int):
                rs = pl.multiple_of(rs, 8)
            return pltpu.make_async_copy(src.at[0, h, pl.ds(rs, nr), :],
                                         kv_v.at[buf(name, h), pl.ds(r0, nr), :], sem)

        def locate(t, j):
            if t is None or isinstance(t, int):
                return None, j if t is None else NP + NS * t + j
            return (t + j // NS, j % NS), NP + j

        def slot_pieces(t, j):
            dyn, gi = locate(t, j)
            if dyn is not None:
                return kv_slot(*dyn), gi
            if gi < NP:
                return pro_slots[gi], gi
            if gi < E1:
                return kv_slot(*divmod(gi - NP, NS)), gi
            return (epi_slots[gi - E1] if gi - E1 < NE else []), gi

        def burst_pieces(t, j):
            dyn, gi = locate(t, j)
            if dyn is not None:
                return kv_burst(*dyn), gi
            if gi < NP:
                return pro_bursts[gi], gi
            if gi < E0:
                return kv_burst(*divmod(gi - NP, NS)), gi
            return (epi_bursts[gi - E0] if gi - E0 < len(epi_bursts) else []), gi

        landed = set()

        def start_slot(t, j):
            pieces, gi = slot_pieces(t, j)
            for pc in pieces:
                copy(pc, sem1.at[gi % NS]).start(priority=LO)

        def start_burst(t, j):
            pieces, gi = burst_pieces(t, j)
            for pc in pieces:
                copy(pc, sem0.at[gi % NS]).start(priority=HI)

        def wait_both(t, j):
            for (pieces, gi), sem in ((slot_pieces(t, j), sem1), (burst_pieces(t, j), sem0)):
                for pc in pieces:
                    copy(pc, sem.at[gi % NS]).wait()
                    if pc[0] in mats:
                        landed.update(_tiles(pc))

        class Jobs:
            def __init__(self):
                self.todo, self.done, self.cool = [], set(), 0

            def add(self, key, need, after, fn):
                self.todo.append((key, _tiles(need), set(after), fn))

            def ready(self):
                return [j for j in self.todo if j[1] <= landed and j[2] <= self.done]

            def run(self, job):
                self.todo.remove(job)
                if not cfg.get("NOJOBS") or job[0] == 0:
                    job[3]()
                self.done.add(job[0])

            def step(self, gap, lo=1, hi=1):
                self.cool -= 1
                ready = self.ready()
                if self.cool <= 0 and len(ready) >= lo:
                    for job in ready[:hi]:
                        self.run(job)
                    self.cool = gap

            def flush(self):
                while self.todo:
                    self.run(self.ready()[0])

        x_cp = pltpu.make_async_copy(x_hbm, x_v, sem_x.at[0])
        wr_cp = pltpu.make_async_copy(wr_hbm, wr_v, sem_x.at[1])
        start_slot(None, 0)
        x_cp.start(priority=HI)
        wr_cp.start(priority=HI)
        for i in range(NS):
            if i > 0:
                start_slot(None, i)
            if i < N0:
                start_burst(None, i)

        x_cp.wait()
        wr_cp.wait()
        x = x_v[0].astype(f32)
        mu = jnp.mean(x, axis=-1, keepdims=True)
        xc = x - mu
        var = jnp.mean(xc * xc, axis=-1, keepdims=True)
        xn = xc / jnp.sqrt(var + 1e-5)
        xn_b = jnp.broadcast_to(xn, (_M, D)).astype(bf16)
        wr = wr_v[...].astype(f32).reshape(1, D)
        r_gate = jax.nn.sigmoid(jnp.sum(xn * wr, axis=-1, keepdims=True))

        QH = H * DH // 2
        q_seen = [0, 0]

        def q_slab(k, half):
            cols = pl.ds(half * QH, QH)
            part = jnp.dot(xn_b[:, k * 128:(k + 1) * 128], wq_v[pl.ds(k * 128, 128), cols],
                           preferred_element_type=f32)
            if q_seen[half] > 0:
                part = part + qacc_s[:, cols]
            q_seen[half] += 1
            if q_seen[half] < D // 128:
                qacc_s[:, cols] = part
            else:
                qb = part.astype(bf16)
                for hh in range(H // 2):
                    q_s[half * (H // 2) + hh] = qb[:, hh * DH:(hh + 1) * DH]

        def gate_piece(c0, n):
            gate_s[:, pl.ds(c0, n)] = lax.dot_general(
                xn_b, wg_v[pl.ds(c0, n), :], _NT, preferred_element_type=f32)

        def up_piece(c0, n):
            up = lax.dot_general(xn_b, wu_v[pl.ds(c0, n), :], _NT, preferred_element_type=f32)
            gate = gate_s[:, pl.ds(c0, n)]
            hid_s[:, pl.ds(c0, n)] = (gate * jax.nn.sigmoid(gate) * up).astype(bf16)

        def down_piece(c0, n):
            y = jnp.dot(hid_s[:, pl.ds(c0, n)], wd_v[pl.ds(c0, n), :],
                        preferred_element_type=f32)[0:1]
            if c0 > 0:
                y = y + g_s[...]
            if c0 + n == F:
                b = xn + (xn * 0.0 + y * r_gate)
                y = b * jax.nn.sigmoid(b)
            g_s[...] = y

        jobs = Jobs()
        for k in range(D // 128):
            for half in range(2):
                jobs.add(("q", k, half), ("wq", 128 * k, 128, half * QH, QH), [],
                         functools.partial(q_slab, k, half))
        for c0 in range(0, F, 256):
            n = min(256, F - c0)
            jobs.add(("g", c0), ("wg", c0, n, 0, D), [], functools.partial(gate_piece, c0, n))
            jobs.add(("u", c0), ("wu", c0, n, 0, D), [("g", c0)], functools.partial(up_piece, c0, n))
        for c0 in range(0, F, 512):
            n = min(512, F - c0)
            after = [("u", c) for c in range(c0, c0 + n, 256)] + ([("d", c0 - 512)] if c0 else [])
            jobs.add(("d", c0), ("wd", c0, n, 0, D), after, functools.partial(down_piece, c0, n))

        for i in range(NP + 2 * NS):
            wait_both(None, i)
            start_burst(None, i + N0)
            start_slot(None, i + NS)
            jobs.step(cfg["JOBGAP"])
        assert not jobs.todo

        def qk(h, anchor):
            m_run = None
            rows = W // cfg["KSUB"]
            for c in range(cfg["KSUB"]):
                s = lax.dot_general(q_s[h], kv_v[buf("K", h), pl.ds(c * rows, rows), :], _NT,
                                    preferred_element_type=f32)
                anchor()
                s_s[:, pl.ds(c * rows, rows)] = s
                for t in range(rows // 128):
                    st = s[:, t * 128:(t + 1) * 128]
                    m_run = st if m_run is None else jnp.maximum(m_run, st)
            return m_run

        def softmax_num(m_run):
            m = jnp.max(m_run, axis=-1, keepdims=True)
            p = jnp.exp((s_s[...] - m) * scale)
            p_s[...] = p.astype(bf16)
            parts = [p[:, t * 128:(t + 1) * 128] for t in range(W // 128)]
            while len(parts) > 1:
                parts = [a + b for a, b in zip(parts[0::2], parts[1::2])]
            return parts[0]

        def pv(h, l_vec, anchor):
            acc = None
            rows = W // cfg["VSUB"]
            for c in range(cfg["VSUB"]):
                o = jnp.dot(p_s[:, pl.ds(c * rows, rows)],
                            kv_v[buf("V", h), pl.ds(c * rows, rows), :], preferred_element_type=f32)
                anchor()
                acc = o if acc is None else o + acc
            l = jnp.sum(l_vec, axis=-1, keepdims=True)
            o_s[h] = (acc / l).astype(bf16)

        def step(t, l_vec, h, j0=0, nslots=NS):
            issued = [0]

            def anchor():
                start_burst(t, j0 + issued[0] + N0)
                issued[0] += 1

            l_new = None
            if cfg.get("NOATT"):
                l_new = jnp.zeros((_M, 128), f32)
            else:
                last = isinstance(h, int) and h == H
                m_run = None if last else qk(h, anchor)
                if l_vec is not None:
                    pv(h - 1, l_vec, anchor)
                if not last:
                    l_new = softmax_num(m_run)
            skip = issued[0]
            for j in range(nslots):
                wait_both(t, j0 + j)
                if j == 0 or j > skip:
                    anchor()
                start_slot(t, j0 + j + NS)
            assert issued[0] == nslots
            return l_new

        l_vec = step(2, None, 0)
        l_vec = lax.fori_loop(3, H - 3, lambda t, l: step(t, l, t - 2), l_vec)
        for t in range(H - 3, H):
            l_vec = step(t, l_vec, t - 2)
        nfull = cfg["KSUB"] + cfg["VSUB"] + 1
        l_vec = step(H, l_vec, H - 2, 0, nfull)
        l_vec = step(H, l_vec, H - 1, nfull, nfull)
        step(H, l_vec, H, 2 * nfull, cfg["VSUB"] + 1)
        j1 = 2 * nfull + cfg["VSUB"] + 1

        out = [None]

        def wo_slab(h):
            part = jnp.dot(o_s[h], wo_v[pl.ds(h * DH, DH), :], preferred_element_type=f32)
            out[0] = part if out[0] is None else part + out[0]

        ojobs = Jobs()
        for h in range(H):
            ojobs.add(h, ("wo", h * DH, DH, 0, D), [], functools.partial(wo_slab, h))
        for j in range(j1, NE):
            wait_both(H, j)
            start_burst(H, j + N0)
            start_slot(H, j + NS)
            if j < NE - 1:
                ojobs.step(2, 2 if j < NE - 6 else 1, 4)
        ojobs.flush()
        out_ref[0] = (x_v[0].astype(f32) + out[0][0:1] * g_s[...]).astype(out_ref.dtype)

    scratch = [
        pltpu.VMEM((1, 1, D), bf16),
        pltpu.VMEM((D,), bf16),
        pltpu.VMEM((D, H * DH), bf16),
        pltpu.VMEM((H * DH, D), bf16),
        pltpu.VMEM((F, D), bf16),
        pltpu.VMEM((F, D), bf16),
        pltpu.VMEM((F, D), bf16),
        pltpu.VMEM((2 * H, W, DH), bf16),
        pltpu.VMEM((_M, H * DH), f32),
        pltpu.VMEM((H, _M, DH), bf16),
        pltpu.VMEM((H, _M, DH), bf16),
        pltpu.VMEM((_M, W), f32),
        pltpu.VMEM((_M, W), bf16),
        pltpu.VMEM((_M, F), f32),
        pltpu.VMEM((_M, F), bf16),
        pltpu.VMEM((1, D), f32),
        pltpu.SemaphoreType.DMA((2,)),
        pltpu.SemaphoreType.DMA((NS,)),
        pltpu.SemaphoreType.DMA((NS,)),
    ]
    return kernel, scratch


@jax.jit
def pallas_recurrent_scan__sliding_block_cached__moe_arch_mod__decode_kernel(
    A_x: jax.Array,
    A_k_cache: jax.Array,
    A_v_cache: jax.Array,
    A_wq: jax.Array,
    A_wo: jax.Array,
    B_x: jax.Array,
    B_w_r: jax.Array,
    B_w_gate: jax.Array,
    B_w_up: jax.Array,
    B_w_down: jax.Array,
):
    del B_x
    _, _, D = A_x.shape
    _, H, SK, DH = A_k_cache.shape
    F = B_w_gate.shape[1]
    W = min(4096, max(256, SK // 4))
    kernel, scratch = _make_kernel(H, SK, W, DH, D, F, CFG)
    any_spec = pl.BlockSpec(memory_space=pl.ANY)
    return pl.pallas_call(
        kernel,
        out_shape=jax.ShapeDtypeStruct(A_x.shape, A_x.dtype),
        in_specs=[any_spec] * 9,
        out_specs=pl.BlockSpec(memory_space=pltpu.VMEM),
        scratch_shapes=scratch,
        compiler_params=pltpu.CompilerParams(
            vmem_limit_bytes=100 * 1024 * 1024,
            disable_bounds_checks=True,
            disable_semaphore_checks=True),
    )(A_x, A_k_cache, A_v_cache, A_wq, A_wo, B_w_r, B_w_gate.T, B_w_up.T, B_w_down)
```

```python
import functools

import jax
import jax.numpy as jnp
from jax import lax
import jax.experimental.pallas as pl
import jax.experimental.pallas.tpu as pltpu

_NT = (((1,), (1,)), ((), ()))
_M = 8

CFG = dict(HI=0, LO=1, N0=14, G_KV=14, G_WQ=14, G_WO=16, G_WG=0, G_WU=16, G_WD=0,
           KSUB=4, VSUB=2, JOBGAP=3, WO_STREAMS=4, R_PRO=2, R_WO=6, NT=4, STAGE=1, END_GAP=8, INIT_EVERY=2)

_BT = 32


def _rects(name, t0, t1, ct):
    out = []
    while t0 < t1:
        r, c = divmod(t0, ct)
        if c or t1 - t0 < ct:
            n = min(ct - c, t1 - t0)
            out.append((name, 8 * r, 8, 128 * c, 128 * n))
            t0 += n
        else:
            rows = (t1 - t0) // ct
            out.append((name, 8 * r, 8 * rows, 0, 128 * ct))
            t0 += rows * ct
    return out


def _split_weight(name, rows, cols, g, reserve):
    ct = cols // 128
    total = rows // 8 * ct
    lo = g % _BT + reserve * _BT
    hi = lo + (total - lo) // _BT * _BT
    blocks = [_rects(name, t, t + _BT, ct) for t in range(lo, hi, _BT)]
    small = [(name, t, ct) for t in list(range(0, lo, 2)) + list(range(hi, total, 2))]
    return blocks, small


def _fit(small, n):
    out, extra, i = [], len(small) - n, 0
    while i < len(small):
        name, t, ct = small[i]
        if extra > 0 and t % 4 == 0 and small[i + 1:i + 2] == [(name, t + 2, ct)] and i % 4 == 0:
            out.append(_rects(name, t, t + 4, ct))
            i, extra = i + 2, extra - 1
        else:
            out.append(_rects(name, t, t + 2, ct))
            i += 1
    assert extra <= 0
    return out + [[]] * (n - len(out))


def _tiles(piece):
    name, r0, nr, c0, nc = piece
    return {(name, r, c) for r in range(r0 // 8, (r0 + nr) // 8) for c in range(c0 // 128, (c0 + nc) // 128)}


def _rotate(*streams):
    out = []
    for i in range(max(len(s) for s in streams)):
        for s in streams:
            out += s[i:i + 1]
    return out


def _make_kernel(H, SK, W, DH, D, F, cfg):
    f32, bf16 = jnp.float32, jnp.bfloat16
    HI, LO, N0 = cfg["HI"], cfg["LO"], cfg["N0"]
    BR = _BT * 8
    G0 = cfg["G_KV"] * 8
    NBLK = (W - G0) // BR
    NS = 2 * NBLK
    scale = DH ** -0.5
    hb = (NBLK + 1) // 2
    border = _rotate(list(range(hb)), list(range(hb, NBLK)))

    tail0 = G0 + NBLK * BR
    n_head = max(1, round(NBLK * G0 / (G0 + W - tail0)))

    def cut(lo, hi, k):
        b = [lo + (hi - lo) // 8 * i // k * 8 for i in range(k + 1)]
        return [(x, y - x) for x, y in zip(b[:-1], b[1:])]
    frag_head, frag_tail = cut(0, G0, n_head), cut(tail0, W, NBLK - n_head)
    frags = ([("V", r, n) for r, n in frag_head] + [("K", r, n) for r, n in frag_head]
             + [("V", r, n) for r, n in frag_tail] + [("K", r, n) for r, n in frag_tail])

    def kv_slot(t, j):
        b0, b1 = border[j // 4], border[(NS + j) // 4]
        row = G0 + BR * b0 + (t & 1) * (BR * (b1 - b0))
        if not isinstance(row, int):
            row = pl.multiple_of(row, 8)
        return [("VK"[j % 2], t ^ ((j % 4) // 2), row, BR)]

    def kv_burst(t, j):
        name, r, n = frags[j]
        return [(name, t + 2, r, n)]

    wq_b, wq_s = _split_weight("wq", D, H * DH, cfg["G_WQ"], cfg["R_PRO"])
    wg_b, wg_s = _split_weight("wg", F, D, cfg["G_WG"], 0)
    wu_b, wu_s = _split_weight("wu", F, D, cfg["G_WU"], 0)
    wd_b, wd_s = _split_weight("wd", F, D, cfg["G_WD"], 0)
    hq, hd = (len(wq_b) + 1) // 2, (len(wd_b) + 1) // 2
    pro_slots = _rotate(wg_b + wd_b[:hd], wq_b[:hq], wu_b + wd_b[hd:], wq_b[hq:])
    NP = len(pro_slots)
    pro_bursts = (_fit(wu_s + wq_s + wg_s + wd_s, NP - 2 * NS)
                  + [kv_burst(t, j) for t in (-2, -1) for j in range(NS)])
    wo_b, wo_s = _split_weight("wo", H * DH, D, cfg["G_WO"], cfg["R_WO"])
    ns = cfg["WO_STREAMS"]
    cuts = [len(wo_b) * i // ns for i in range(ns + 1)]
    epi_slots = _rotate(*[wo_b[a:b][::-1] for a, b in zip(cuts[:-1], cuts[1:])][::-1])[::-1]
    NE = len(epi_slots)
    E1 = NP + NS * H
    E0 = NP + NS * (H - 2)
    NA = cfg["KSUB"] + cfg["VSUB"]
    inside = [N0 + j0 + k for j0, n in ((0, NA), (NS, NA), (2 * NS, NA), (2 * NS + NA + 1, NA),
                                        (2 * NS + 2 * NA + 2, cfg["VSUB"])) for k in range(n)]
    n_b = 2 * NS + NE + N0 - cfg["END_GAP"]
    if cfg["STAGE"]:
        staged = [[("stage", r, 16, c, 128)] for r in range(0, DH, 16) for c in range(0, D, 128)]
        wo_s = [s for s in wo_s if s[1] >= DH // 8 * (D // 128)]
        spare = [i for i in range(n_b) if i not in inside][:len(staged) - len(inside)]
        where = dict(zip(sorted(inside + spare), staged))
        plain = iter(_fit(wo_s, n_b - len(staged)))
        epi_bursts = [where[i] if i in where else next(plain) for i in range(n_b)]
    else:
        epi_bursts = _fit(wo_s, n_b)
    vpu_rows = [(blk[0][1], blk[0][2]) for blk in epi_slots[NE - cfg["NT"]:]]
    assert all(len(blk) == 1 for blk in epi_slots[NE - cfg["NT"]:])

    def kernel(x_hbm, k_hbm, v_hbm, wq_hbm, wo_hbm, wr_hbm, wg_hbm, wu_hbm, wd_hbm,
               out_ref,
               x_v, wr_v, wq_v, wo_v, wg_v, wu_v, wd_v, kv_v,
               qacc_s, q_s, o_s, s_s, p_s, gate_s, hid_s, g_s,
               ob_s, sems):
        mats = dict(wq=(wq_hbm, wq_v), wo=(wo_hbm, wo_v), wg=(wg_hbm, wg_v), wu=(wu_hbm, wu_v),
                    wd=(wd_hbm, wd_v))

        def buf(name, h):
            return h + (H if name == "V" else 0)

        def copy(piece, sem):
            if piece[0] == "stage":
                _, r0, nr, c0, nc = piece
                return pltpu.make_async_copy(wo_hbm.at[pl.ds(r0, nr), pl.ds(c0, nc)],
                                             kv_v.at[2 * H, pl.ds(c0 + r0, nr), :], sem)
            if piece[0] in mats:
                name, r0, nr, c0, nc = piece
                src, dst = mats[name]
                return pltpu.make_async_copy(src.at[pl.ds(r0, nr), pl.ds(c0, nc)],
                                             dst.at[pl.ds(r0, nr), pl.ds(c0, nc)], sem)
            name, h, r0, nr = piece
            src = k_hbm if name == "K" else v_hbm
            rs = SK - W + r0
            if not isinstance(rs, int):
                rs = pl.multiple_of(rs, 8)
            return pltpu.make_async_copy(src.at[0, h, pl.ds(rs, nr), :],
                                         kv_v.at[buf(name, h), pl.ds(r0, nr), :], sem)

        def locate(t, j):
            if t is None or isinstance(t, int):
                return None, j if t is None else NP + NS * t + j
            return (t + j // NS, j % NS), NP + j

        def slot_pieces(t, j):
            dyn, gi = locate(t, j)
            if dyn is not None:
                return kv_slot(*dyn), gi
            if gi < NP:
                return pro_slots[gi], gi
            if gi < E1:
                return kv_slot(*divmod(gi - NP, NS)), gi
            return (epi_slots[gi - E1] if gi - E1 < NE else []), gi

        def burst_pieces(t, j):
            dyn, gi = locate(t, j)
            if dyn is not None:
                return kv_burst(*dyn), gi
            if gi < NP:
                return pro_bursts[gi], gi
            if gi < E0:
                return kv_burst(*divmod(gi - NP, NS)), gi
            return (epi_bursts[gi - E0] if gi - E0 < len(epi_bursts) else []), gi

        landed = set()

        def start_slot(t, j):
            pieces, gi = slot_pieces(t, j)
            for pc in pieces:
                copy(pc, sems.at[gi % NS]).start(priority=LO)

        def start_burst(t, j):
            pieces, gi = burst_pieces(t, j)
            for pc in pieces:
                copy(pc, sems.at[NS + gi % NS]).start(priority=HI)

        def wait_pieces(pieces, sem):
            for pc in pieces:
                copy(pc, sem).wait()
                if pc[0] not in "KV":
                    landed.update(_tiles(pc))

        def wait_slot(t, j):
            pieces, gi = slot_pieces(t, j)
            wait_pieces(pieces, sems.at[gi % NS])

        def wait_burst(t, j):
            pieces, gi = burst_pieces(t, j)
            wait_pieces(pieces, sems.at[NS + gi % NS])

        def wait_both(t, j):
            wait_slot(t, j)
            wait_burst(t, j)

        class Jobs:
            def __init__(self):
                self.todo, self.done, self.cool = [], set(), 0

            def add(self, key, need, after, fn):
                self.todo.append((key, _tiles(need), set(after), fn))

            def ready(self):
                return [j for j in self.todo if j[1] <= landed and j[2] <= self.done]

            def run(self, job):
                self.todo.remove(job)
                if not cfg.get("NOJOBS") or job[0] == 0:
                    job[3]()
                self.done.add(job[0])

            def step(self, gap, lo=1, hi=1):
                self.cool -= 1
                ready = self.ready()
                if self.cool <= 0 and len(ready) >= lo:
                    for job in ready[:hi]:
                        self.run(job)
                    self.cool = gap

            def flush(self):
                while self.todo:
                    self.run(self.ready()[0])

        x_cp = pltpu.make_async_copy(x_hbm, x_v, sems.at[2 * NS])
        wr_cp = pltpu.make_async_copy(wr_hbm, wr_v, sems.at[2 * NS + 1])
        start_slot(None, 0)
        x_cp.start(priority=HI)
        wr_cp.start(priority=HI)
        nb = 0
        for i in range(1, NS):
            start_slot(None, i)
            if i % cfg["INIT_EVERY"] == 0 and nb < N0:
                start_burst(None, nb)
                nb += 1
        for i in range(nb, N0):
            start_burst(None, i)

        def plain_slot(t, j):
            wait_both(t, j)
            start_burst(t, j + N0)
            start_slot(t, j + NS)

        x_cp.wait()
        wr_cp.wait()
        plain_slot(None, 0)
        x = x_v[0].astype(f32)
        mu = jnp.mean(x, axis=-1, keepdims=True)
        xc = x - mu
        plain_slot(None, 1)
        var = jnp.mean(xc * xc, axis=-1, keepdims=True)
        xn = xc / jnp.sqrt(var + 1e-5)
        xn_b = jnp.broadcast_to(xn, (_M, D)).astype(bf16)
        plain_slot(None, 2)
        plain_slot(None, 3)
        wr = wr_v[...].astype(f32).reshape(1, D)
        r_gate = jax.nn.sigmoid(jnp.sum(xn * wr, axis=-1, keepdims=True))

        QH = H * DH // 2
        q_seen = [0, 0]

        def q_slab(k, half):
            cols = pl.ds(half * QH, QH)
            part = jnp.dot(xn_b[:, k * 128:(k + 1) * 128], wq_v[pl.ds(k * 128, 128), cols],
                           preferred_element_type=f32)
            if q_seen[half] > 0:
                part = part + qacc_s[:, cols]
            q_seen[half] += 1
            if q_seen[half] < D // 128:
                qacc_s[:, cols] = part
            else:
                qb = part.astype(bf16)
                for hh in range(H // 2):
                    q_s[half * (H // 2) + hh] = qb[:, hh * DH:(hh + 1) * DH]

        def gate_piece(c0, n):
            gate_s[:, pl.ds(c0, n)] = lax.dot_general(
                xn_b, wg_v[pl.ds(c0, n), :], _NT, preferred_element_type=f32)

        def up_piece(c0, n):
            up = lax.dot_general(xn_b, wu_v[pl.ds(c0, n), :], _NT, preferred_element_type=f32)
            gate = gate_s[:, pl.ds(c0, n)]
            hid_s[:, pl.ds(c0, n)] = (gate * jax.nn.sigmoid(gate) * up).astype(bf16)

        def down_piece(c0, n):
            y = jnp.dot(hid_s[:, pl.ds(c0, n)], wd_v[pl.ds(c0, n), :],
                        preferred_element_type=f32)[0:1]
            if c0 > 0:
                y = y + g_s[...]
            if c0 + n == F:
                b = xn + (xn * 0.0 + y * r_gate)
                y = b * jax.nn.sigmoid(b)
            g_s[...] = y

        jobs = Jobs()
        for k in range(D // 128):
            for half in range(2):
                jobs.add(("q", k, half), ("wq", 128 * k, 128, half * QH, QH), [],
                         functools.partial(q_slab, k, half))
        for c0 in range(0, F, 256):
            n = min(256, F - c0)
            jobs.add(("g", c0), ("wg", c0, n, 0, D), [], functools.partial(gate_piece, c0, n))
            jobs.add(("u", c0), ("wu", c0, n, 0, D), [("g", c0)], functools.partial(up_piece, c0, n))
        for c0 in range(0, F, 512):
            n = min(512, F - c0)
            after = [("u", c) for c in range(c0, c0 + n, 256)] + ([("d", c0 - 512)] if c0 else [])
            jobs.add(("d", c0), ("wd", c0, n, 0, D), after, functools.partial(down_piece, c0, n))

        for i in range(4, NP + 2 * NS):
            plain_slot(None, i)
            jobs.step(cfg["JOBGAP"])
        assert not jobs.todo

        def qk(h, anchor):
            m_run = None
            rows = W // cfg["KSUB"]
            for c in range(cfg["KSUB"]):
                s = lax.dot_general(q_s[h], kv_v[buf("K", h), pl.ds(c * rows, rows), :], _NT,
                                    preferred_element_type=f32)
                anchor()
                s_s[:, pl.ds(c * rows, rows)] = s
                for t in range(rows // 128):
                    st = s[:, t * 128:(t + 1) * 128]
                    m_run = st if m_run is None else jnp.maximum(m_run, st)
            return m_run

        def softmax_num(m_run):
            m = jnp.max(m_run, axis=-1, keepdims=True)
            p = jnp.exp((s_s[...] - m) * scale)
            p_s[...] = p.astype(bf16)
            parts = [p[:, t * 128:(t + 1) * 128] for t in range(W // 128)]
            while len(parts) > 1:
                parts = [a + b for a, b in zip(parts[0::2], parts[1::2])]
            return parts[0]

        def pv(h, l_vec, anchor):
            acc = None
            rows = W // cfg["VSUB"]
            for c in range(cfg["VSUB"]):
                o = jnp.dot(p_s[:, pl.ds(c * rows, rows)],
                            kv_v[buf("V", h), pl.ds(c * rows, rows), :], preferred_element_type=f32)
                anchor()
                acc = o if acc is None else o + acc
            l = jnp.sum(l_vec, axis=-1, keepdims=True)
            o_s[h] = (acc / l).astype(bf16)

        def step(t, l_vec, h, j0=0, nslots=NS):
            issued = [0]

            def anchor():
                start_burst(t, j0 + issued[0] + N0)
                issued[0] += 1

            l_new = None
            if cfg.get("NOATT"):
                l_new = jnp.zeros((_M, 128), f32)
            else:
                last = isinstance(h, int) and h == H
                m_run = None if last else qk(h, anchor)
                if l_vec is not None:
                    pv(h - 1, l_vec, anchor)
                if not last:
                    l_new = softmax_num(m_run)
            skip = issued[0]
            for j in range(nslots):
                wait_both(t, j0 + j)
                if j == 0 or j > skip:
                    anchor()
                start_slot(t, j0 + j + NS)
            assert issued[0] == nslots
            return l_new

        l_vec = step(2, None, 0)
        l_vec = lax.fori_loop(3, H - 3, lambda t, l: step(t, l, t - 2), l_vec)
        for t in range(H - 3, H):
            l_vec = step(t, l_vec, t - 2)
        nfull = cfg["KSUB"] + cfg["VSUB"] + 1
        l_vec = step(H, l_vec, H - 2, 0, nfull)
        l_vec = step(H, l_vec, H - 1, nfull, nfull)
        step(H, l_vec, H, 2 * nfull, cfg["VSUB"] + 1)
        j1 = 2 * nfull + cfg["VSUB"] + 1

        out = [None]

        def accumulate(part):
            out[0] = part if out[0] is None else part + out[0]

        def wo_rows(h, a, b):
            accumulate(jnp.dot(o_s[h][:, a:b], wo_v[pl.ds(h * DH + a, b - a), :],
                               preferred_element_type=f32))

        def wo_staged():
            accumulate(jnp.concatenate(
                [jnp.dot(o_s[0], kv_v[2 * H, pl.ds(c, DH), :], preferred_element_type=f32)
                 for c in range(0, D, 128)], axis=1))

        def spread_o():
            cols = {}
            for i, (r0, n) in enumerate(vpu_rows):
                for r in range(r0, r0 + n, 32):
                    h, a = divmod(r, DH)
                    if h not in cols:
                        row = o_s[h][0:1].astype(f32)
                        cols[h] = jnp.broadcast_to(row, (128, DH)).T
                    ob_s[i, pl.ds(r - r0, 32), :] = cols[h][a:a + 32]

        def wo_vpu(i, acc):
            r0, n = vpu_rows[i]
            w = wo_v[pl.ds(r0, n), :].astype(f32)
            ob = ob_s[i]
            prod = w * jnp.concatenate([ob] * (D // 128), axis=1)
            parts = [prod[r:r + 8] for r in range(0, n, 8)] + ([] if acc is None else [acc])
            while len(parts) > 1:
                parts = [a + b for a, b in zip(parts[0::2], parts[1::2])] + parts[len(parts) & ~1:]
            return parts[0]

        ojobs = Jobs()
        late = {r for r0, n in vpu_rows for r in range(r0, r0 + n, 8)}
        for h in range(H):
            if h == 0 and cfg["STAGE"]:
                ojobs.add(0, ("stage", 0, DH, 0, D), [], wo_staged)
                continue
            a = None
            for r in range(0, DH + 8, 8):
                free = r < DH and h * DH + r not in late
                if free and a is None:
                    a = r
                if not free and a is not None:
                    ojobs.add((h, a), ("wo", h * DH + a, r - a, 0, D), [],
                              functools.partial(wo_rows, h, a, r))
                    a = None
        if vpu_rows:
            spread_o()
        nxt = j1
        last_mxu = NE - cfg["NT"] - 1
        for j in range(j1, last_mxu + 1):
            wait_slot(H, j)
            upto = j + 1 if j < last_mxu else n_b - 2 * NS
            upto = max(upto, min(j + N0 - cfg["END_GAP"] + cfg["NT"] + 1 - (last_mxu - j) * 2, n_b - 2 * NS))
            while nxt < upto:
                wait_burst(H, nxt)
                nxt += 1
            start_burst(H, j + N0)
            start_slot(H, j + NS)
            if j < last_mxu:
                ojobs.step(2, 2 if j < last_mxu - 4 else 1, 4)
        ojobs.flush()
        acc = None
        base = x_v[0].astype(f32) + out[0][0:1] * g_s[...]
        for i in range(cfg["NT"]):
            wait_slot(H, last_mxu + 1 + i)
            acc = wo_vpu(i, acc)
        if acc is not None:
            base = base + jnp.sum(acc, axis=0, keepdims=True) * g_s[...]
        out_ref[0] = base.astype(out_ref.dtype)

    scratch = [
        pltpu.VMEM((1, 1, D), bf16),
        pltpu.VMEM((D,), bf16),
        pltpu.VMEM((D, H * DH), bf16),
        pltpu.VMEM((H * DH, D), bf16),
        pltpu.VMEM((F, D), bf16),
        pltpu.VMEM((F, D), bf16),
        pltpu.VMEM((F, D), bf16),
        pltpu.VMEM((2 * H + 1, W, DH), bf16),
        pltpu.VMEM((_M, H * DH), f32),
        pltpu.VMEM((H, _M, DH), bf16),
        pltpu.VMEM((H, _M, DH), bf16),
        pltpu.VMEM((_M, W), f32),
        pltpu.VMEM((_M, W), bf16),
        pltpu.VMEM((_M, F), f32),
        pltpu.VMEM((_M, F), bf16),
        pltpu.VMEM((1, D), f32),
        pltpu.VMEM((max(1, cfg["NT"]), _BT * 1024 // D, 128), f32),
        pltpu.SemaphoreType.DMA((2 * NS + 2,)),
    ]
    return kernel, scratch


@jax.jit
def pallas_recurrent_scan__sliding_block_cached__moe_arch_mod__decode_kernel(
    A_x: jax.Array,
    A_k_cache: jax.Array,
    A_v_cache: jax.Array,
    A_wq: jax.Array,
    A_wo: jax.Array,
    B_x: jax.Array,
    B_w_r: jax.Array,
    B_w_gate: jax.Array,
    B_w_up: jax.Array,
    B_w_down: jax.Array,
):
    del B_x
    _, _, D = A_x.shape
    _, H, SK, DH = A_k_cache.shape
    F = B_w_gate.shape[1]
    W = min(4096, max(256, SK // 4))
    kernel, scratch = _make_kernel(H, SK, W, DH, D, F, CFG)
    any_spec = pl.BlockSpec(memory_space=pl.ANY)
    return pl.pallas_call(
        kernel,
        out_shape=jax.ShapeDtypeStruct(A_x.shape, A_x.dtype),
        in_specs=[any_spec] * 9,
        out_specs=pl.BlockSpec(memory_space=pltpu.VMEM),
        scratch_shapes=scratch,
        compiler_params=pltpu.CompilerParams(
            vmem_limit_bytes=100 * 1024 * 1024,
            disable_bounds_checks=True,
            disable_semaphore_checks=True),
    )(A_x, A_k_cache, A_v_cache, A_wq, A_wo, B_w_r, B_w_gate.T, B_w_up.T, B_w_down)
```

```python
import functools

import jax
import jax.numpy as jnp
from jax import lax
import jax.experimental.pallas as pl
import jax.experimental.pallas.tpu as pltpu

_NT = (((1,), (1,)), ((), ()))
_M = 8
_BT = 32

CFG = dict(
    N0=14,
    G_KV=14, G_WQ=14, G_WO=16, G_WG=0, G_WU=16, G_WD=0,
    KSUB=4, VSUB=2,
    JOBGAP=3, WO_STREAMS=4, R_PRO=2, R_WO=6, NT=8, INIT_EVERY=2)


def _rects(name, t0, t1, ct):
    out = []
    while t0 < t1:
        r, c = divmod(t0, ct)
        if c or t1 - t0 < ct:
            n = min(ct - c, t1 - t0)
            out.append((name, 8 * r, 8, 128 * c, 128 * n))
            t0 += n
        else:
            rows = (t1 - t0) // ct
            out.append((name, 8 * r, 8 * rows, 0, 128 * ct))
            t0 += rows * ct
    return out


def _split_weight(name, rows, cols, g, reserve):
    ct = cols // 128
    total = rows // 8 * ct
    lo = g % _BT + reserve * _BT
    hi = lo + (total - lo) // _BT * _BT
    blocks = [_rects(name, t, t + _BT, ct) for t in range(lo, hi, _BT)]
    small = [(name, t, ct) for t in list(range(0, lo, 2)) + list(range(hi, total, 2))]
    return blocks, small


def _fit(small, n):
    out, extra, i = [], len(small) - n, 0
    while i < len(small):
        name, t, ct = small[i]
        if extra > 0 and t % 4 == 0 and small[i + 1:i + 2] == [(name, t + 2, ct)] and i % 4 == 0:
            out.append(_rects(name, t, t + 4, ct))
            i, extra = i + 2, extra - 1
        else:
            out.append(_rects(name, t, t + 2, ct))
            i += 1
    assert extra <= 0
    return out + [[]] * (n - len(out))


def _tiles(piece):
    name, r0, nr, c0, nc = piece
    return {(name, r, c) for r in range(r0 // 8, (r0 + nr) // 8)
            for c in range(c0 // 128, (c0 + nc) // 128)}


def _rotate(*streams):
    out = []
    for i in range(max(len(s) for s in streams)):
        for s in streams:
            out += s[i:i + 1]
    return out


def _tree_sum(parts):
    while len(parts) > 1:
        parts = [a + b for a, b in zip(parts[0::2], parts[1::2])] + parts[len(parts) & ~1:]
    return parts[0]


class _Jobs:
    def __init__(self, landed):
        self.landed, self.todo, self.done, self.cool = landed, [], set(), 0

    def add(self, key, need, after, fn):
        self.todo.append((key, _tiles(need), set(after), fn))

    def ready(self):
        return [j for j in self.todo if j[1] <= self.landed and j[2] <= self.done]

    def run(self, job):
        self.todo.remove(job)
        job[3]()
        self.done.add(job[0])

    def step(self, gap, lo=1, hi=1):
        self.cool -= 1
        ready = self.ready()
        if self.cool <= 0 and len(ready) >= lo:
            for job in ready[:hi]:
                self.run(job)
            self.cool = gap

    def flush(self):
        while self.todo:
            self.run(self.ready()[0])


def _make_kernel(H, SK, W, DH, D, F, cfg):
    f32, bf16 = jnp.float32, jnp.bfloat16
    HI, LO = 0, 1
    N0, NT, KSUB, VSUB = cfg["N0"], cfg["NT"], cfg["KSUB"], cfg["VSUB"]
    BR = _BT * 8
    G0 = cfg["G_KV"] * 8
    NBLK = (W - G0) // BR
    NS = 2 * NBLK
    NA = KSUB + VSUB
    scale = DH ** -0.5
    assert DH == 128 and H % 2 == 0 and NS % 4 == 2 and N0 + NA < NS

    hb = (NBLK + 1) // 2
    border = _rotate(list(range(hb)), list(range(hb, NBLK)))
    tail0 = G0 + NBLK * BR
    n_head = max(1, round(NBLK * G0 / (G0 + W - tail0)))

    def cut(lo, hi, k):
        b = [lo + (hi - lo) // 8 * i // k * 8 for i in range(k + 1)]
        return [(x, y - x) for x, y in zip(b[:-1], b[1:])]
    frags = [(name, r, n) for part in (cut(0, G0, n_head), cut(tail0, W, NBLK - n_head))
             for name in "VK" for r, n in part]

    def kv_slot(t, j):
        i = (t % 2) * NS + j
        return [("VK"[i % 2], t - t % 2 + (i % 4) // 2, G0 + BR * border[i // 4], BR)]

    def kv_burst(t, j):
        name, r, n = frags[j]
        return [(name, t + 2, r, n)]

    wq_b, wq_s = _split_weight("wq", D, H * DH, cfg["G_WQ"], cfg["R_PRO"])
    wg_b, wg_s = _split_weight("wg", F, D, cfg["G_WG"], 0)
    wu_b, wu_s = _split_weight("wu", F, D, cfg["G_WU"], 0)
    wd_b, wd_s = _split_weight("wd", F, D, cfg["G_WD"], 0)
    hq, hd = (len(wq_b) + 1) // 2, (len(wd_b) + 1) // 2
    pro_slots = _rotate(wg_b + wd_b[:hd], wq_b[:hq], wu_b + wd_b[hd:], wq_b[hq:])
    NP = len(pro_slots)
    pro_bursts = _fit(wu_s + wq_s + wg_s + wd_s, NP - 2 * NS)

    wo_b, wo_s = _split_weight("wo", H * DH, D, cfg["G_WO"], cfg["R_WO"])
    cuts = [len(wo_b) * i // cfg["WO_STREAMS"] for i in range(cfg["WO_STREAMS"] + 1)]
    epi_slots = _rotate(*[wo_b[a:b][::-1] for a, b in zip(cuts[:-1], cuts[1:])][::-1])[::-1]
    NE = len(epi_slots)
    inside = [N0 + j0 + k for j0, n in ((0, NA), (NS, NA), (2 * NS, NA), (2 * NS + NA + 1, NA),
                                        (2 * NS + 2 * NA + 2, VSUB)) for k in range(n)]
    staged = [[("stage", r, 16, c, 128)] for r in range(0, DH, 16) for c in range(0, D, 128)]
    wo_s = [s for s in wo_s if s[1] >= DH // 8 * (D // 128)]
    n_b = len(staged) + len(wo_s)
    spare = [i for i in range(n_b) if i not in inside][:len(staged) - len(inside)]
    where = dict(zip(sorted(inside + spare), staged))
    plain = iter(_fit(wo_s, len(wo_s)))
    epi_bursts = [where[i] if i in where else next(plain) for i in range(n_b)]
    vpu_rows = [(blk[0][1], blk[0][2]) for blk in epi_slots[NE - NT:]]
    assert all(len(blk) == 1 for blk in epi_slots[NE - NT:])
    assert n_b - 2 * NS - N0 + 6 <= NE - NT and NT < NS

    def slot_pieces(i):
        if i < 0:
            return pro_slots[NP + i]
        if i < NS * H:
            return kv_slot(*divmod(i, NS))
        return epi_slots[i - NS * H] if i - NS * H < NE else []

    def burst_pieces(i):
        if i < -2 * NS:
            return pro_bursts[NP + i]
        if i < NS * (H - 2):
            return kv_burst(*divmod(i, NS))
        return epi_bursts[i - NS * (H - 2)] if i - NS * (H - 2) < n_b else []

    def kernel(x_hbm, k_hbm, v_hbm, wq_hbm, wo_hbm, wr_hbm, wg_hbm, wu_hbm, wd_hbm,
               out_ref,
               x_v, wr_v, wq_v, wo_v, wg_v, wu_v, wd_v, kv_v,
               qacc_s, q_s, o_s, s_s, p_s, gate_s, hid_s, g_s, ob_s, sems):
        mats = dict(wq=(wq_hbm, wq_v), wo=(wo_hbm, wo_v), wg=(wg_hbm, wg_v), wu=(wu_hbm, wu_v),
                    wd=(wd_hbm, wd_v))
        landed = set()

        def copy(piece, sem, dh):
            if piece[0] in "KV":
                name, h, r0, nr = piece
                src = k_hbm if name == "K" else v_hbm
                return pltpu.make_async_copy(
                    src.at[0, h + dh, pl.ds(SK - W + r0, nr), :],
                    kv_v.at[h + dh + (H if name == "V" else 0), pl.ds(r0, nr), :], sem)
            name, r0, nr, c0, nc = piece
            if name == "stage":
                return pltpu.make_async_copy(wo_hbm.at[pl.ds(r0, nr), pl.ds(c0, nc)],
                                             kv_v.at[2 * H, pl.ds(c0 + r0, nr), :], sem)
            src, dst = mats[name]
            return pltpu.make_async_copy(src.at[pl.ds(r0, nr), pl.ds(c0, nc)],
                                         dst.at[pl.ds(r0, nr), pl.ds(c0, nc)], sem)

        def start_slot(i, dh=0):
            for pc in slot_pieces(i):
                copy(pc, sems.at[i % NS], dh).start(priority=LO)

        def start_burst(i, dh=0):
            for pc in burst_pieces(i):
                copy(pc, sems.at[NS + i % NS], dh).start(priority=HI)

        def wait_pieces(pieces, sem, dh):
            for pc in pieces:
                copy(pc, sem, dh).wait()
            for pc in pieces:
                if pc[0] not in "KV":
                    landed.update(_tiles(pc))

        def wait_slot(i, dh=0):
            wait_pieces(slot_pieces(i), sems.at[i % NS], dh)

        def wait_burst(i, dh=0):
            wait_pieces(burst_pieces(i), sems.at[NS + i % NS], dh)

        def plain_slot(i):
            wait_slot(i)
            wait_burst(i)
            start_burst(i + N0)
            start_slot(i + NS)

        x_cp = pltpu.make_async_copy(x_hbm, x_v, sems.at[2 * NS])
        wr_cp = pltpu.make_async_copy(wr_hbm, wr_v, sems.at[2 * NS + 1])
        start_slot(-NP)
        x_cp.start(priority=HI)
        wr_cp.start(priority=HI)
        nb = 0
        for i in range(1, NS):
            start_slot(-NP + i)
            if i % cfg["INIT_EVERY"] == 0 and nb < N0:
                start_burst(-NP + nb)
                nb += 1
        for i in range(nb, N0):
            start_burst(-NP + i)

        x_cp.wait()
        wr_cp.wait()
        plain_slot(-NP)
        x = x_v[0].astype(f32)
        mu = jnp.mean(x, axis=-1, keepdims=True)
        xc = x - mu
        plain_slot(-NP + 1)
        var = jnp.mean(xc * xc, axis=-1, keepdims=True)
        xn = xc / jnp.sqrt(var + 1e-5)
        xn_b = jnp.broadcast_to(xn, (_M, D)).astype(bf16)
        plain_slot(-NP + 2)
        plain_slot(-NP + 3)
        wr = wr_v[...].astype(f32).reshape(1, D)
        r_gate = jax.nn.sigmoid(jnp.sum(xn * wr, axis=-1, keepdims=True))

        QH = H * DH // 2
        q_seen = [0, 0]

        def q_slab(k, half):
            cols = pl.ds(half * QH, QH)
            part = jnp.dot(xn_b[:, k * 128:(k + 1) * 128], wq_v[pl.ds(k * 128, 128), cols],
                           preferred_element_type=f32)
            if q_seen[half] > 0:
                part = part + qacc_s[:, cols]
            q_seen[half] += 1
            if q_seen[half] < D // 128:
                qacc_s[:, cols] = part
            else:
                qb = part.astype(bf16)
                for hh in range(H // 2):
                    q_s[half * (H // 2) + hh] = qb[:, hh * DH:(hh + 1) * DH]

        def gate_piece(c0, n):
            gate_s[:, pl.ds(c0, n)] = lax.dot_general(
                xn_b, wg_v[pl.ds(c0, n), :], _NT, preferred_element_type=f32)

        def up_piece(c0, n):
            up = lax.dot_general(xn_b, wu_v[pl.ds(c0, n), :], _NT, preferred_element_type=f32)
            gate = gate_s[:, pl.ds(c0, n)]
            hid_s[:, pl.ds(c0, n)] = (gate * jax.nn.sigmoid(gate) * up).astype(bf16)

        def down_piece(c0, n):
            y = jnp.dot(hid_s[:, pl.ds(c0, n)], wd_v[pl.ds(c0, n), :],
                        preferred_element_type=f32)[0:1]
            if c0 > 0:
                y = y + g_s[...]
            if c0 + n == F:
                b = xn + (xn * 0.0 + y * r_gate)
                y = b * jax.nn.sigmoid(b)
            g_s[...] = y

        jobs = _Jobs(landed)
        for k in range(D // 128):
            for half in range(2):
                jobs.add(("q", k, half), ("wq", 128 * k, 128, half * QH, QH), [],
                         functools.partial(q_slab, k, half))
        for c0 in range(0, F, 256):
            n = min(256, F - c0)
            jobs.add(("g", c0), ("wg", c0, n, 0, D), [], functools.partial(gate_piece, c0, n))
            jobs.add(("u", c0), ("wu", c0, n, 0, D), [("g", c0)], functools.partial(up_piece, c0, n))
        for c0 in range(0, F, 512):
            n = min(512, F - c0)
            after = [("u", c) for c in range(c0, c0 + n, 256)] + ([("d", c0 - 512)] if c0 else [])
            jobs.add(("d", c0), ("wd", c0, n, 0, D), after, functools.partial(down_piece, c0, n))

        for i in range(-NP + 4, 2 * NS):
            plain_slot(i)
            jobs.step(cfg["JOBGAP"])
        assert not jobs.todo

        def qk(h, burst):
            m_run = None
            rows = W // KSUB
            for c in range(KSUB):
                s = lax.dot_general(q_s[h], kv_v[h, pl.ds(c * rows, rows), :], _NT,
                                    preferred_element_type=f32)
                burst()
                s_s[:, pl.ds(c * rows, rows)] = s
                for t in range(rows // 128):
                    st = s[:, t * 128:(t + 1) * 128]
                    m_run = st if m_run is None else jnp.maximum(m_run, st)
            return m_run

        def softmax_num(m_run):
            m = jnp.max(m_run, axis=-1, keepdims=True)
            p = jnp.exp((s_s[...] - m) * scale)
            p_s[...] = p.astype(bf16)
            return _tree_sum([p[:, t * 128:(t + 1) * 128] for t in range(W // 128)])

        def pv(h, l_vec, burst):
            acc = None
            rows = W // VSUB
            for c in range(VSUB):
                o = jnp.dot(p_s[:, pl.ds(c * rows, rows)], kv_v[H + h, pl.ds(c * rows, rows), :],
                            preferred_element_type=f32)
                burst()
                acc = o if acc is None else o + acc
            l = jnp.sum(l_vec, axis=-1, keepdims=True)
            o_s[h] = (acc / l).astype(bf16)

        def step(h, l_vec, i0, nslots, dh=0):
            issued = [0]

            def burst():
                start_burst(i0 + issued[0] + N0, dh)
                issued[0] += 1

            m_run = qk(h + dh, burst) if h < H else None
            if h > 0:
                pv(h - 1 + dh, l_vec, burst)
            l_new = softmax_num(m_run) if h < H else None
            early = issued[0]
            for j in range(nslots):
                wait_slot(i0 + j, dh)
                wait_burst(i0 + j, dh)
                if j == 0 or j > early:
                    burst()
                start_slot(i0 + j + NS, dh)
            assert issued[0] == nslots
            return l_new

        def two_steps(p, l_vec):
            l_vec = step(1, l_vec, 3 * NS, NS, 2 * p)
            return step(2, l_vec, 4 * NS, NS, 2 * p)

        l_vec = step(0, None, 2 * NS, NS)
        l_vec = lax.fori_loop(0, (H - 6) // 2, two_steps, l_vec)
        for h in range(H - 5, H - 2):
            l_vec = step(h, l_vec, (h + 2) * NS, NS)
        e0 = H * NS
        l_vec = step(H - 2, l_vec, e0, NA + 1)
        l_vec = step(H - 1, l_vec, e0 + NA + 1, NA + 1)
        step(H, l_vec, e0 + 2 * NA + 2, VSUB + 1)

        out = [None]

        def accumulate(part):
            out[0] = part if out[0] is None else part + out[0]

        def wo_rows(h, a, b):
            accumulate(jnp.dot(o_s[h][:, a:b], wo_v[pl.ds(h * DH + a, b - a), :],
                               preferred_element_type=f32))

        def wo_staged():
            accumulate(jnp.concatenate(
                [jnp.dot(o_s[0], kv_v[2 * H, pl.ds(c, DH), :], preferred_element_type=f32)
                 for c in range(0, D, 128)], axis=1))

        ojobs = _Jobs(landed)
        ojobs.add(0, ("stage", 0, DH, 0, D), [], wo_staged)
        late = {r for r0, n in vpu_rows for r in range(r0, r0 + n, 8)}
        for h in range(1, H):
            a = None
            for r in range(0, DH + 8, 8):
                free = r < DH and h * DH + r not in late
                if free and a is None:
                    a = r
                if not free and a is not None:
                    ojobs.add((h, a), ("wo", h * DH + a, r - a, 0, D), [],
                              functools.partial(wo_rows, h, a, r))
                    a = None

        cols = {}
        for i, (r0, n) in enumerate(vpu_rows):
            for r in range(r0, r0 + n, 32):
                h, a = divmod(r, DH)
                if h not in cols:
                    cols[h] = jnp.broadcast_to(o_s[h][0:1].astype(f32), (128, DH)).T
                ob_s[i, pl.ds(r - r0, 32), :] = cols[h][a:a + 32]

        last_mxu = e0 + NE - NT - 1
        for i in range(e0 + 2 * NA + VSUB + 3, last_mxu + 1):
            plain_slot(i)
            if i < last_mxu:
                ojobs.step(2, 2 if i < last_mxu - 4 else 1, 4)
        for i in range(last_mxu + 1, (H - 2) * NS + n_b):
            wait_burst(i)
        ojobs.flush()
        base = x_v[0].astype(f32) + out[0][0:1] * g_s[...]
        acc = []
        for i, (r0, n) in enumerate(vpu_rows):
            wait_slot(last_mxu + 1 + i)
            prod = (wo_v[pl.ds(r0, n), :].astype(f32)
                    * jnp.concatenate([ob_s[i]] * (D // 128), axis=1))
            acc = [_tree_sum([prod[r:r + 8] for r in range(0, n, 8)] + acc)]
        res = base + jnp.sum(acc[0], axis=0, keepdims=True) * g_s[...]
        out_ref[0] = res.astype(out_ref.dtype)

    scratch = [
        pltpu.VMEM((1, 1, D), bf16),
        pltpu.VMEM((D,), bf16),
        pltpu.VMEM((D, H * DH), bf16),
        pltpu.VMEM((H * DH, D), bf16),
        pltpu.VMEM((F, D), bf16),
        pltpu.VMEM((F, D), bf16),
        pltpu.VMEM((F, D), bf16),
        pltpu.VMEM((2 * H + 1, W, DH), bf16),
        pltpu.VMEM((_M, H * DH), f32),
        pltpu.VMEM((H, _M, DH), bf16),
        pltpu.VMEM((H, _M, DH), bf16),
        pltpu.VMEM((_M, W), f32),
        pltpu.VMEM((_M, W), bf16),
        pltpu.VMEM((_M, F), f32),
        pltpu.VMEM((_M, F), bf16),
        pltpu.VMEM((1, D), f32),
        pltpu.VMEM((NT, _BT * 1024 // D, 128), f32),
        pltpu.SemaphoreType.DMA((2 * NS + 2,)),
    ]
    return kernel, scratch


@jax.jit
def pallas_recurrent_scan__sliding_block_cached__moe_arch_mod__decode_kernel(
    A_x: jax.Array,
    A_k_cache: jax.Array,
    A_v_cache: jax.Array,
    A_wq: jax.Array,
    A_wo: jax.Array,
    B_x: jax.Array,
    B_w_r: jax.Array,
    B_w_gate: jax.Array,
    B_w_up: jax.Array,
    B_w_down: jax.Array,
):
    del B_x
    _, _, D = A_x.shape
    _, H, SK, DH = A_k_cache.shape
    F = B_w_gate.shape[1]
    W = min(4096, max(256, SK // 4))
    kernel, scratch = _make_kernel(H, SK, W, DH, D, F, CFG)
    any_spec = pl.BlockSpec(memory_space=pl.ANY)
    return pl.pallas_call(
        kernel,
        out_shape=jax.ShapeDtypeStruct(A_x.shape, A_x.dtype),
        in_specs=[any_spec] * 9,
        out_specs=pl.BlockSpec(memory_space=pltpu.VMEM),
        scratch_shapes=scratch,
        compiler_params=pltpu.CompilerParams(
            vmem_limit_bytes=100 * 1024 * 1024,
            disable_bounds_checks=True,
            disable_semaphore_checks=True),
    )(A_x, A_k_cache, A_v_cache, A_wq, A_wo, B_w_r, B_w_gate.T, B_w_up.T, B_w_down)
```

```python
import functools

import jax
import jax.numpy as jnp
import numpy as np
from jax import lax
import jax.experimental.pallas as pl
import jax.experimental.pallas.tpu as pltpu

_NT = (((1,), (1,)), ((), ()))
_M = 8
_BT = 32

CFG = dict(
    N0=14,
    G_KV=14, G_WQ=14, G_WO=16, G_WG=0, G_WU=16, G_WD=0,
    KSUB=4, VSUB=2,
    JOBGAP=3, WO_STREAMS=4, R_PRO=2, R_WO=6, NT=8, INIT_EVERY=2)


def _rects(name, t0, t1, ct):
    out = []
    while t0 < t1:
        r, c = divmod(t0, ct)
        if c or t1 - t0 < ct:
            n = min(ct - c, t1 - t0)
            out.append((name, 8 * r, 8, 128 * c, 128 * n))
            t0 += n
        else:
            rows = (t1 - t0) // ct
            out.append((name, 8 * r, 8 * rows, 0, 128 * ct))
            t0 += rows * ct
    return out


def _split_weight(name, rows, cols, g, reserve):
    ct = cols // 128
    total = rows // 8 * ct
    lo = g % _BT + reserve * _BT
    hi = lo + (total - lo) // _BT * _BT
    blocks = [_rects(name, t, t + _BT, ct) for t in range(lo, hi, _BT)]
    small = [(name, t, ct) for t in list(range(0, lo, 2)) + list(range(hi, total, 2))]
    return blocks, small


def _fit(small, n):
    out, extra, i = [], len(small) - n, 0
    while i < len(small):
        name, t, ct = small[i]
        if extra > 0 and t % 4 == 0 and small[i + 1:i + 2] == [(name, t + 2, ct)] and i % 4 == 0:
            out.append(_rects(name, t, t + 4, ct))
            i, extra = i + 2, extra - 1
        else:
            out.append(_rects(name, t, t + 2, ct))
            i += 1
    assert extra <= 0
    return out + [[]] * (n - len(out))


def _tiles(piece):
    name, r0, nr, c0, nc = piece
    return {(name, r, c) for r in range(r0 // 8, (r0 + nr) // 8)
            for c in range(c0 // 128, (c0 + nc) // 128)}


def _rotate(*streams):
    out = []
    for i in range(max(len(s) for s in streams)):
        for s in streams:
            out += s[i:i + 1]
    return out


def _tree_sum(parts):
    while len(parts) > 1:
        parts = [a + b for a, b in zip(parts[0::2], parts[1::2])] + parts[len(parts) & ~1:]
    return parts[0]


def _rb(v):
    return v.astype(jnp.bfloat16).astype(jnp.float32)


class _Jobs:
    def __init__(self, landed):
        self.landed, self.todo, self.done, self.cool = landed, [], set(), 0

    def add(self, key, need, after, fn):
        self.todo.append((key, _tiles(need), set(after), fn))

    def ready(self):
        return [j for j in self.todo if j[1] <= self.landed and j[2] <= self.done]

    def run(self, job):
        self.todo.remove(job)
        job[3]()
        self.done.add(job[0])

    def step(self, gap, lo=1, hi=1):
        self.cool -= 1
        ready = self.ready()
        if self.cool <= 0 and len(ready) >= lo:
            for job in ready[:hi]:
                self.run(job)
            self.cool = gap

    def flush(self):
        while self.todo:
            self.run(self.ready()[0])


def _make_kernel(H, SK, W, DH, D, F, cfg):
    f32, bf16 = jnp.float32, jnp.bfloat16
    HI, LO = 0, 1
    N0, NT, KSUB, VSUB = cfg["N0"], cfg["NT"], cfg["KSUB"], cfg["VSUB"]
    BR = _BT * 8
    G0 = cfg["G_KV"] * 8
    NBLK = (W - G0) // BR
    NS = 2 * NBLK
    NA = KSUB + VSUB
    scale = float(np.asarray(DH ** -0.5, bf16))
    eps = float(np.asarray(1e-5, bf16))
    assert DH == 128 and H % 2 == 0 and NS % 4 == 2 and N0 + NA < NS

    hb = (NBLK + 1) // 2
    border = _rotate(list(range(hb)), list(range(hb, NBLK)))
    tail0 = G0 + NBLK * BR
    n_head = max(1, round(NBLK * G0 / (G0 + W - tail0)))

    def cut(lo, hi, k):
        b = [lo + (hi - lo) // 8 * i // k * 8 for i in range(k + 1)]
        return [(x, y - x) for x, y in zip(b[:-1], b[1:])]
    frags = [(name, r, n) for part in (cut(0, G0, n_head), cut(tail0, W, NBLK - n_head))
             for name in "VK" for r, n in part]

    def kv_slot(t, j):
        i = (t % 2) * NS + j
        return [("VK"[i % 2], t - t % 2 + (i % 4) // 2, G0 + BR * border[i // 4], BR)]

    def kv_burst(t, j):
        name, r, n = frags[j]
        return [(name, t + 2, r, n)]

    wq_b, wq_s = _split_weight("wq", D, H * DH, cfg["G_WQ"], cfg["R_PRO"])
    wg_b, wg_s = _split_weight("wg", F, D, cfg["G_WG"], 0)
    wu_b, wu_s = _split_weight("wu", F, D, cfg["G_WU"], 0)
    wd_b, wd_s = _split_weight("wd", F, D, cfg["G_WD"], 0)
    hq, hd = (len(wq_b) + 1) // 2, (len(wd_b) + 1) // 2
    pro_slots = _rotate(wg_b + wd_b[:hd], wq_b[:hq], wu_b + wd_b[hd:], wq_b[hq:])
    NP = len(pro_slots)
    pro_bursts = _fit(wu_s + wq_s + wg_s + wd_s, NP - 2 * NS)

    wo_b, wo_s = _split_weight("wo", H * DH, D, cfg["G_WO"], cfg["R_WO"])
    cuts = [len(wo_b) * i // cfg["WO_STREAMS"] for i in range(cfg["WO_STREAMS"] + 1)]
    epi_slots = _rotate(*[wo_b[a:b][::-1] for a, b in zip(cuts[:-1], cuts[1:])][::-1])[::-1]
    NE = len(epi_slots)
    inside = [N0 + j0 + k for j0, n in ((0, NA), (NS, NA), (2 * NS, NA), (2 * NS + NA + 1, NA),
                                        (2 * NS + 2 * NA + 2, VSUB)) for k in range(n)]
    staged = [[("stage", r, 16, c, 128)] for r in range(0, DH, 16) for c in range(0, D, 128)]
    wo_s = [s for s in wo_s if s[1] >= DH // 8 * (D // 128)]
    n_b = len(staged) + len(wo_s)
    spare = [i for i in range(n_b) if i not in inside][:len(staged) - len(inside)]
    where = dict(zip(sorted(inside + spare), staged))
    plain = iter(_fit(wo_s, len(wo_s)))
    epi_bursts = [where[i] if i in where else next(plain) for i in range(n_b)]
    vpu_rows = [(blk[0][1], blk[0][2]) for blk in epi_slots[NE - NT:]]
    assert all(len(blk) == 1 for blk in epi_slots[NE - NT:])
    assert n_b - 2 * NS - N0 + 6 <= NE - NT and NT < NS

    def slot_pieces(i):
        if i < 0:
            return pro_slots[NP + i]
        if i < NS * H:
            return kv_slot(*divmod(i, NS))
        return epi_slots[i - NS * H] if i - NS * H < NE else []

    def burst_pieces(i):
        if i < -2 * NS:
            return pro_bursts[NP + i]
        if i < NS * (H - 2):
            return kv_burst(*divmod(i, NS))
        return epi_bursts[i - NS * (H - 2)] if i - NS * (H - 2) < n_b else []

    def kernel(x_hbm, k_hbm, v_hbm, wq_hbm, wo_hbm, wr_hbm, wg_hbm, wu_hbm, wd_hbm,
               out_ref,
               x_v, wr_v, wq_v, wo_v, wg_v, wu_v, wd_v, kv_v,
               qacc_s, q_s, o_s, s_s, p_s, gate_s, hid_s, g_s, ob_s, sems):
        mats = dict(wq=(wq_hbm, wq_v), wo=(wo_hbm, wo_v), wg=(wg_hbm, wg_v), wu=(wu_hbm, wu_v),
                    wd=(wd_hbm, wd_v))
        landed = set()

        def copy(piece, sem, dh):
            if piece[0] in "KV":
                name, h, r0, nr = piece
                src = k_hbm if name == "K" else v_hbm
                return pltpu.make_async_copy(
                    src.at[0, h + dh, pl.ds(SK - W + r0, nr), :],
                    kv_v.at[h + dh + (H if name == "V" else 0), pl.ds(r0, nr), :], sem)
            name, r0, nr, c0, nc = piece
            if name == "stage":
                return pltpu.make_async_copy(wo_hbm.at[pl.ds(r0, nr), pl.ds(c0, nc)],
                                             kv_v.at[2 * H, pl.ds(c0 + r0, nr), :], sem)
            src, dst = mats[name]
            return pltpu.make_async_copy(src.at[pl.ds(r0, nr), pl.ds(c0, nc)],
                                         dst.at[pl.ds(r0, nr), pl.ds(c0, nc)], sem)

        def start_slot(i, dh=0):
            for pc in slot_pieces(i):
                copy(pc, sems.at[i % NS], dh).start(priority=LO)

        def start_burst(i, dh=0):
            for pc in burst_pieces(i):
                copy(pc, sems.at[NS + i % NS], dh).start(priority=HI)

        def wait_pieces(pieces, sem, dh):
            for pc in pieces:
                copy(pc, sem, dh).wait()
            for pc in pieces:
                if pc[0] not in "KV":
                    landed.update(_tiles(pc))

        def wait_slot(i, dh=0):
            wait_pieces(slot_pieces(i), sems.at[i % NS], dh)

        def wait_burst(i, dh=0):
            wait_pieces(burst_pieces(i), sems.at[NS + i % NS], dh)

        def plain_slot(i):
            wait_slot(i)
            wait_burst(i)
            start_burst(i + N0)
            start_slot(i + NS)

        x_cp = pltpu.make_async_copy(x_hbm, x_v, sems.at[2 * NS])
        wr_cp = pltpu.make_async_copy(wr_hbm, wr_v, sems.at[2 * NS + 1])
        start_slot(-NP)
        x_cp.start(priority=HI)
        wr_cp.start(priority=HI)
        nb = 0
        for i in range(1, NS):
            start_slot(-NP + i)
            if i % cfg["INIT_EVERY"] == 0 and nb < N0:
                start_burst(-NP + nb)
                nb += 1
        for i in range(nb, N0):
            start_burst(-NP + i)

        x_cp.wait()
        wr_cp.wait()
        plain_slot(-NP)
        x = x_v[0].astype(f32)
        mu = jnp.mean(x, axis=-1, keepdims=True)
        xc = x - mu
        plain_slot(-NP + 1)
        var = jnp.mean(xc * xc, axis=-1, keepdims=True)
        xn = _rb(_rb(x - _rb(mu)) / _rb(jnp.sqrt(_rb(_rb(var) + eps))))
        xn_b = jnp.broadcast_to(xn, (_M, D)).astype(bf16)
        plain_slot(-NP + 2)
        plain_slot(-NP + 3)
        wr = wr_v[...].astype(f32).reshape(1, D)
        r_gate = _rb(jax.nn.sigmoid(_rb(jnp.sum(xn * wr, axis=-1, keepdims=True))))

        QH = H * DH // 2
        q_seen = [0, 0]

        def q_slab(k, half):
            cols = pl.ds(half * QH, QH)
            part = jnp.dot(xn_b[:, k * 128:(k + 1) * 128], wq_v[pl.ds(k * 128, 128), cols],
                           preferred_element_type=f32)
            if q_seen[half] > 0:
                part = part + qacc_s[:, cols]
            q_seen[half] += 1
            if q_seen[half] < D // 128:
                qacc_s[:, cols] = part
            else:
                qb = part.astype(bf16)
                for hh in range(H // 2):
                    q_s[half * (H // 2) + hh] = qb[:, hh * DH:(hh + 1) * DH]

        def gate_piece(c0, n):
            gate_s[:, pl.ds(c0, n)] = lax.dot_general(
                xn_b, wg_v[pl.ds(c0, n), :], _NT, preferred_element_type=f32)

        def up_piece(c0, n):
            up = lax.dot_general(xn_b, wu_v[pl.ds(c0, n), :], _NT, preferred_element_type=f32)
            gate = _rb(gate_s[:, pl.ds(c0, n)])
            hid_s[:, pl.ds(c0, n)] = (_rb(gate * jax.nn.sigmoid(gate)) * _rb(up)).astype(bf16)

        def down_piece(c0, n):
            y = jnp.dot(hid_s[:, pl.ds(c0, n)], wd_v[pl.ds(c0, n), :],
                        preferred_element_type=f32)[0:1]
            if c0 > 0:
                y = y + g_s[...]
            if c0 + n == F:
                b = _rb(xn + (xn * 0.0 + _rb(_rb(y) * r_gate)))
                y = _rb(b * jax.nn.sigmoid(b))
            g_s[...] = y

        jobs = _Jobs(landed)
        for k in range(D // 128):
            for half in range(2):
                jobs.add(("q", k, half), ("wq", 128 * k, 128, half * QH, QH), [],
                         functools.partial(q_slab, k, half))
        for c0 in range(0, F, 256):
            n = min(256, F - c0)
            jobs.add(("g", c0), ("wg", c0, n, 0, D), [], functools.partial(gate_piece, c0, n))
            jobs.add(("u", c0), ("wu", c0, n, 0, D), [("g", c0)], functools.partial(up_piece, c0, n))
        for c0 in range(0, F, 512):
            n = min(512, F - c0)
            after = [("u", c) for c in range(c0, c0 + n, 256)] + ([("d", c0 - 512)] if c0 else [])
            jobs.add(("d", c0), ("wd", c0, n, 0, D), after, functools.partial(down_piece, c0, n))

        for i in range(-NP + 4, 2 * NS):
            plain_slot(i)
            jobs.step(cfg["JOBGAP"])
        assert not jobs.todo

        def qk(h, burst):
            m_run = None
            rows = W // KSUB
            for c in range(KSUB):
                s = lax.dot_general(q_s[h], kv_v[h, pl.ds(c * rows, rows), :], _NT,
                                    preferred_element_type=f32)
                burst()
                s = _rb(_rb(s) * scale)
                s_s[:, pl.ds(c * rows, rows)] = s
                for t in range(rows // 128):
                    st = s[:, t * 128:(t + 1) * 128]
                    m_run = st if m_run is None else jnp.maximum(m_run, st)
            return m_run

        def softmax_num(m_run):
            m = jnp.max(m_run, axis=-1, keepdims=True)
            p = jnp.exp(s_s[...] - m)
            p_s[...] = p.astype(bf16)
            return _tree_sum([p[:, t * 128:(t + 1) * 128] for t in range(W // 128)])

        def pv(h, l_vec, burst):
            acc = None
            rows = W // VSUB
            for c in range(VSUB):
                o = jnp.dot(p_s[:, pl.ds(c * rows, rows)], kv_v[H + h, pl.ds(c * rows, rows), :],
                            preferred_element_type=f32)
                burst()
                acc = o if acc is None else o + acc
            l = jnp.sum(l_vec, axis=-1, keepdims=True)
            o_s[h] = (acc / l).astype(bf16)

        def step(h, l_vec, i0, nslots, dh=0):
            issued = [0]

            def burst():
                start_burst(i0 + issued[0] + N0, dh)
                issued[0] += 1

            m_run = qk(h + dh, burst) if h < H else None
            if h > 0:
                pv(h - 1 + dh, l_vec, burst)
            l_new = softmax_num(m_run) if h < H else None
            early = issued[0]
            for j in range(nslots):
                wait_slot(i0 + j, dh)
                wait_burst(i0 + j, dh)
                if j == 0 or j > early:
                    burst()
                start_slot(i0 + j + NS, dh)
            assert issued[0] == nslots
            return l_new

        def two_steps(p, l_vec):
            l_vec = step(1, l_vec, 3 * NS, NS, 2 * p)
            return step(2, l_vec, 4 * NS, NS, 2 * p)

        l_vec = step(0, None, 2 * NS, NS)
        l_vec = lax.fori_loop(0, (H - 6) // 2, two_steps, l_vec)
        for h in range(H - 5, H - 2):
            l_vec = step(h, l_vec, (h + 2) * NS, NS)
        e0 = H * NS
        l_vec = step(H - 2, l_vec, e0, NA + 1)
        l_vec = step(H - 1, l_vec, e0 + NA + 1, NA + 1)
        step(H, l_vec, e0 + 2 * NA + 2, VSUB + 1)

        out = [None]

        def accumulate(part):
            out[0] = part if out[0] is None else part + out[0]

        def wo_rows(h, a, b):
            accumulate(jnp.dot(o_s[h][:, a:b], wo_v[pl.ds(h * DH + a, b - a), :],
                               preferred_element_type=f32))

        def wo_staged():
            accumulate(jnp.concatenate(
                [jnp.dot(o_s[0], kv_v[2 * H, pl.ds(c, DH), :], preferred_element_type=f32)
                 for c in range(0, D, 128)], axis=1))

        ojobs = _Jobs(landed)
        ojobs.add(0, ("stage", 0, DH, 0, D), [], wo_staged)
        late = {r for r0, n in vpu_rows for r in range(r0, r0 + n, 8)}
        for h in range(1, H):
            a = None
            for r in range(0, DH + 8, 8):
                free = r < DH and h * DH + r not in late
                if free and a is None:
                    a = r
                if not free and a is not None:
                    ojobs.add((h, a), ("wo", h * DH + a, r - a, 0, D), [],
                              functools.partial(wo_rows, h, a, r))
                    a = None

        cols = {}
        for i, (r0, n) in enumerate(vpu_rows):
            for r in range(r0, r0 + n, 32):
                h, a = divmod(r, DH)
                if h not in cols:
                    cols[h] = jnp.broadcast_to(o_s[h][0:1].astype(f32), (128, DH)).T
                ob_s[i, pl.ds(r - r0, 32), :] = cols[h][a:a + 32]

        last_mxu = e0 + NE - NT - 1
        for i in range(e0 + 2 * NA + VSUB + 3, last_mxu + 1):
            plain_slot(i)
            if i < last_mxu:
                ojobs.step(2, 2 if i < last_mxu - 4 else 1, 4)
        for i in range(last_mxu + 1, (H - 2) * NS + n_b):
            wait_burst(i)
        ojobs.flush()
        row0 = lax.broadcasted_iota(jnp.int32, (_M, D), 0) == 0
        acc = [jnp.where(row0, out[0], 0.0)]
        for i, (r0, n) in enumerate(vpu_rows):
            wait_slot(last_mxu + 1 + i)
            prod = (wo_v[pl.ds(r0, n), :].astype(f32)
                    * jnp.concatenate([ob_s[i]] * (D // 128), axis=1))
            acc = [_tree_sum([prod[r:r + 8] for r in range(0, n, 8)] + acc)]
        attn = _rb(jnp.sum(acc[0], axis=0, keepdims=True))
        out_ref[0] = (x_v[0].astype(f32) + _rb(attn * g_s[...])).astype(out_ref.dtype)

    scratch = [
        pltpu.VMEM((1, 1, D), bf16),
        pltpu.VMEM((D,), bf16),
        pltpu.VMEM((D, H * DH), bf16),
        pltpu.VMEM((H * DH, D), bf16),
        pltpu.VMEM((F, D), bf16),
        pltpu.VMEM((F, D), bf16),
        pltpu.VMEM((F, D), bf16),
        pltpu.VMEM((2 * H + 1, W, DH), bf16),
        pltpu.VMEM((_M, H * DH), f32),
        pltpu.VMEM((H, _M, DH), bf16),
        pltpu.VMEM((H, _M, DH), bf16),
        pltpu.VMEM((_M, W), f32),
        pltpu.VMEM((_M, W), bf16),
        pltpu.VMEM((_M, F), f32),
        pltpu.VMEM((_M, F), bf16),
        pltpu.VMEM((1, D), f32),
        pltpu.VMEM((NT, _BT * 1024 // D, 128), f32),
        pltpu.SemaphoreType.DMA((2 * NS + 2,)),
    ]
    return kernel, scratch


@jax.jit
def pallas_recurrent_scan__sliding_block_cached__moe_arch_mod__decode_kernel(
    A_x: jax.Array,
    A_k_cache: jax.Array,
    A_v_cache: jax.Array,
    A_wq: jax.Array,
    A_wo: jax.Array,
    B_x: jax.Array,
    B_w_r: jax.Array,
    B_w_gate: jax.Array,
    B_w_up: jax.Array,
    B_w_down: jax.Array,
):
    del B_x
    _, _, D = A_x.shape
    _, H, SK, DH = A_k_cache.shape
    F = B_w_gate.shape[1]
    W = min(4096, max(256, SK // 4))
    kernel, scratch = _make_kernel(H, SK, W, DH, D, F, CFG)
    any_spec = pl.BlockSpec(memory_space=pl.ANY)
    return pl.pallas_call(
        kernel,
        out_shape=jax.ShapeDtypeStruct(A_x.shape, A_x.dtype),
        in_specs=[any_spec] * 9,
        out_specs=pl.BlockSpec(memory_space=pltpu.VMEM),
        scratch_shapes=scratch,
        compiler_params=pltpu.CompilerParams(
            vmem_limit_bytes=100 * 1024 * 1024,
            disable_bounds_checks=True,
            disable_semaphore_checks=True),
    )(A_x, A_k_cache, A_v_cache, A_wq, A_wo, B_w_r, B_w_gate.T, B_w_up.T, B_w_down)
```

```python
import functools

import jax
import jax.numpy as jnp
import numpy as np
from jax import lax
import jax.experimental.pallas as pl
import jax.experimental.pallas.tpu as pltpu

_NT = (((1,), (1,)), ((), ()))
_M = 8
_BT = 32

CFG = dict(
    N0=14,
    G_KV=14, G_WQ=14, G_WO=14, G_WG=0, G_WU=16, G_WD=0,
    KSUB=4, VSUB=2,
    JOBGAP=3, WO_STREAMS=6, R_PRO=2, R_WO=6, UNITS=48, INIT_EVERY=2)


def _rects(name, t0, t1, ct):
    out = []
    while t0 < t1:
        r, c = divmod(t0, ct)
        if c or t1 - t0 < ct:
            n = min(ct - c, t1 - t0)
            out.append((name, 8 * r, 8, 128 * c, 128 * n))
            t0 += n
        else:
            rows = (t1 - t0) // ct
            out.append((name, 8 * r, 8 * rows, 0, 128 * ct))
            t0 += rows * ct
    return out


def _split_weight(name, rows, cols, g, reserve):
    ct = cols // 128
    total = rows // 8 * ct
    lo = g % _BT + reserve * _BT
    hi = lo + (total - lo) // _BT * _BT
    blocks = [_rects(name, t, t + _BT, ct) for t in range(lo, hi, _BT)]
    small = [(name, t, ct) for t in list(range(0, lo, 2)) + list(range(hi, total, 2))]
    return blocks, small


def _fit(small, n):
    out, extra, i = [], len(small) - n, 0
    while i < len(small):
        name, t, ct = small[i]
        if extra > 0 and t % 4 == 0 and small[i + 1:i + 2] == [(name, t + 2, ct)] and i % 4 == 0:
            out.append(_rects(name, t, t + 4, ct))
            i, extra = i + 2, extra - 1
        else:
            out.append(_rects(name, t, t + 2, ct))
            i += 1
    assert extra <= 0
    return out + [[]] * (n - len(out))


def _tiles(piece):
    name, r0, nr, c0, nc = piece
    return {(name, r, c) for r in range(r0 // 8, (r0 + nr) // 8)
            for c in range(c0 // 128, (c0 + nc) // 128)}


def _rotate(*streams):
    out = []
    for i in range(max(len(s) for s in streams)):
        for s in streams:
            out += s[i:i + 1]
    return out


def _tree_sum(parts):
    while len(parts) > 1:
        parts = [a + b for a, b in zip(parts[0::2], parts[1::2])] + parts[len(parts) & ~1:]
    return parts[0]


def _rb(v):
    return v.astype(jnp.bfloat16).astype(jnp.float32)


class _Jobs:
    def __init__(self, landed):
        self.landed, self.todo, self.done, self.cool = landed, [], set(), 0

    def add(self, key, need, after, fn):
        self.todo.append((key, _tiles(need), set(after), fn))

    def ready(self):
        return [j for j in self.todo if j[1] <= self.landed and j[2] <= self.done]

    def run(self, job):
        self.todo.remove(job)
        job[3]()
        self.done.add(job[0])

    def step(self, gap):
        self.cool -= 1
        ready = self.ready()
        if self.cool <= 0 and ready:
            self.run(ready[0])
            self.cool = gap


def _make_kernel(H, SK, W, DH, D, F, cfg):
    f32, bf16 = jnp.float32, jnp.bfloat16
    HI, LO = 0, 1
    N0, KSUB, VSUB = cfg["N0"], cfg["KSUB"], cfg["VSUB"]
    BR = _BT * 8
    G0 = cfg["G_KV"] * 8
    NBLK = (W - G0) // BR
    NS = 2 * NBLK
    NA = KSUB + VSUB
    scale = float(np.asarray(DH ** -0.5, bf16))
    eps = float(np.asarray(1e-5, bf16))
    assert DH == 128 and H % 2 == 0 and NS % 4 == 2 and N0 + NA < NS

    hb = (NBLK + 1) // 2
    border = _rotate(list(range(hb)), list(range(hb, NBLK)))
    tail0 = G0 + NBLK * BR
    n_head = max(1, round(NBLK * G0 / (G0 + W - tail0)))

    def cut(lo, hi, k):
        b = [lo + (hi - lo) // 8 * i // k * 8 for i in range(k + 1)]
        return [(x, y - x) for x, y in zip(b[:-1], b[1:])]
    frags = [(name, r, n) for part in (cut(0, G0, n_head), cut(tail0, W, NBLK - n_head))
             for name in "VK" for r, n in part]

    def kv_slot(t, j):
        i = (t % 2) * NS + j
        return [("VK"[i % 2], t - t % 2 + (i % 4) // 2, G0 + BR * border[i // 4], BR)]

    def kv_burst(t, j):
        name, r, n = frags[j]
        return [(name, t + 2, r, n)]

    wq_b, wq_s = _split_weight("wq", D, H * DH, cfg["G_WQ"], cfg["R_PRO"])
    wg_b, wg_s = _split_weight("wg", F, D, cfg["G_WG"], 0)
    wu_b, wu_s = _split_weight("wu", F, D, cfg["G_WU"], 0)
    wd_b, wd_s = _split_weight("wd", F, D, cfg["G_WD"], 0)
    q1, q2 = (len(wq_b) + 2) // 3, (2 * len(wq_b) + 2) // 3
    pro_slots = _rotate(wg_b, wq_b[:q1], wu_b, wq_b[q1:q2], wd_b, wq_b[q2:])
    NP = len(pro_slots)
    pro_bursts = _fit(wu_s + wq_s + wg_s + wd_s, NP - 2 * NS)

    UPR = D // 256
    UB = _BT // 2
    UPH = DH // 8 * UPR
    n_units = H * UPH
    u_lo = cfg["G_WO"] // 2 + cfg["R_WO"] * UB
    u_hi = u_lo + (n_units - u_lo) // UB * UB
    wo_b = [[("wo", u, UB)] for u in range(u_lo, u_hi, UB)]
    wo_s = [[("wo", u, 1)] for u in list(range(UPH, u_lo)) + list(range(u_hi, n_units))]
    cuts = [len(wo_b) * i // cfg["WO_STREAMS"] for i in range(cfg["WO_STREAMS"] + 1)]
    epi_slots = _rotate(*[wo_b[a:b][::-1] for a, b in zip(cuts[:-1], cuts[1:])][::-1])[::-1]
    NE = len(epi_slots)
    inside = [N0 + j0 + k for j0, n in ((0, NA), (NS, NA), (2 * NS, NA), (2 * NS + NA + 1, NA),
                                        (2 * NS + 2 * NA + 2, VSUB)) for k in range(n)]
    staged = [[("stage", r, 16, c, 128)] for r in range(0, DH, 16) for c in range(0, D, 128)]
    n_b = len(staged) + len(wo_s)
    assert n_b <= 2 * NS + NE
    spare = [i for i in range(n_b) if i not in inside][:len(staged) - len(inside)]
    where = dict(zip(sorted(inside + spare), staged))
    plain = iter(wo_s)
    epi_bursts = [where[i] if i in where else next(plain) for i in range(n_b)]

    def slot_pieces(i):
        if i < 0:
            return pro_slots[NP + i]
        if i < NS * H:
            return kv_slot(*divmod(i, NS))
        return epi_slots[i - NS * H] if i - NS * H < NE else []

    def burst_pieces(i):
        if i < -2 * NS:
            return pro_bursts[NP + i]
        if i < NS * (H - 2):
            return kv_burst(*divmod(i, NS))
        return epi_bursts[i - NS * (H - 2)] if i - NS * (H - 2) < n_b else []

    def kernel(x_hbm, k_hbm, v_hbm, wq_hbm, wo_hbm, wou_hbm, wr_hbm, wg_hbm, wu_hbm, wd_hbm,
               out_ref,
               x_v, wr_v, wq_v, wo_v, wg_v, wu_v, wd_v, kv_v,
               qacc_s, q_s, o_s, s_s, p_s, gate_s, hid_s, g_s, ob_s, sems):
        mats = dict(wq=(wq_hbm, wq_v), wg=(wg_hbm, wg_v), wu=(wu_hbm, wu_v), wd=(wd_hbm, wd_v))
        landed = set()
        wo_landed = []

        def copy(piece, sem, dh):
            if piece[0] in "KV":
                name, h, r0, nr = piece
                src = k_hbm if name == "K" else v_hbm
                return pltpu.make_async_copy(
                    src.at[0, h + dh, pl.ds(SK - W + r0, nr), :],
                    kv_v.at[h + dh + (H if name == "V" else 0), pl.ds(r0, nr), :], sem)
            if piece[0] == "wo":
                _, u, n = piece
                return pltpu.make_async_copy(wou_hbm.at[pl.ds(u, n)], wo_v.at[pl.ds(u, n)], sem)
            name, r0, nr, c0, nc = piece
            if name == "stage":
                return pltpu.make_async_copy(wo_hbm.at[pl.ds(r0, nr), pl.ds(c0, nc)],
                                             kv_v.at[2 * H, pl.ds(c0 + r0, nr), :], sem)
            src, dst = mats[name]
            return pltpu.make_async_copy(src.at[pl.ds(r0, nr), pl.ds(c0, nc)],
                                         dst.at[pl.ds(r0, nr), pl.ds(c0, nc)], sem)

        def start_slot(i, dh=0):
            for pc in slot_pieces(i):
                copy(pc, sems.at[i % NS], dh).start(priority=LO)

        def start_burst(i, dh=0):
            for pc in burst_pieces(i):
                copy(pc, sems.at[NS + i % NS], dh).start(priority=HI)

        def wait_pieces(pieces, sem, dh):
            for pc in pieces:
                copy(pc, sem, dh).wait()
            for pc in pieces:
                if pc[0] == "wo":
                    wo_landed.append(pc[1:])
                elif pc[0] not in "KV":
                    landed.update(_tiles(pc))

        def wait_slot(i, dh=0):
            wait_pieces(slot_pieces(i), sems.at[i % NS], dh)

        def wait_burst(i, dh=0):
            wait_pieces(burst_pieces(i), sems.at[NS + i % NS], dh)

        def plain_slot(i):
            wait_slot(i)
            wait_burst(i)
            start_burst(i + N0)
            start_slot(i + NS)

        x_cp = pltpu.make_async_copy(x_hbm, x_v, sems.at[2 * NS])
        wr_cp = pltpu.make_async_copy(wr_hbm, wr_v, sems.at[2 * NS + 1])
        start_slot(-NP)
        x_cp.start(priority=HI)
        wr_cp.start(priority=HI)
        nb = 0
        for i in range(1, NS):
            start_slot(-NP + i)
            if i % cfg["INIT_EVERY"] == 0 and nb < N0:
                start_burst(-NP + nb)
                nb += 1
        for i in range(nb, N0):
            start_burst(-NP + i)

        x_cp.wait()
        wr_cp.wait()
        plain_slot(-NP)
        x = x_v[0].astype(f32)
        mu = jnp.mean(x, axis=-1, keepdims=True)
        xc = x - mu
        plain_slot(-NP + 1)
        var = jnp.mean(xc * xc, axis=-1, keepdims=True)
        xn = _rb(_rb(x - _rb(mu)) / _rb(jnp.sqrt(_rb(_rb(var) + eps))))
        xn_b = jnp.broadcast_to(xn, (_M, D)).astype(bf16)
        plain_slot(-NP + 2)
        plain_slot(-NP + 3)
        wr = wr_v[...].astype(f32).reshape(1, D)
        r_gate = _rb(jax.nn.sigmoid(_rb(jnp.sum(xn * wr, axis=-1, keepdims=True))))

        QH = H * DH // 2
        q_seen = [0, 0]

        def q_slab(k, half):
            cols = pl.ds(half * QH, QH)
            part = jnp.dot(xn_b[:, k * 128:(k + 1) * 128], wq_v[pl.ds(k * 128, 128), cols],
                           preferred_element_type=f32)
            if q_seen[half] > 0:
                part = part + qacc_s[:, cols]
            q_seen[half] += 1
            if q_seen[half] < D // 128:
                qacc_s[:, cols] = part
            else:
                qb = part.astype(bf16)
                for hh in range(H // 2):
                    q_s[half * (H // 2) + hh] = qb[:, hh * DH:(hh + 1) * DH]

        def gate_piece(c0, n):
            gate_s[:, pl.ds(c0, n)] = lax.dot_general(
                xn_b, wg_v[pl.ds(c0, n), :], _NT, preferred_element_type=f32)

        def up_piece(c0, n):
            up = lax.dot_general(xn_b, wu_v[pl.ds(c0, n), :], _NT, preferred_element_type=f32)
            gate = _rb(gate_s[:, pl.ds(c0, n)])
            hid_s[:, pl.ds(c0, n)] = (_rb(gate * jax.nn.sigmoid(gate)) * _rb(up)).astype(bf16)

        def down_piece(c0, n):
            y = jnp.dot(hid_s[:, pl.ds(c0, n)], wd_v[pl.ds(c0, n), :],
                        preferred_element_type=f32)[0:1]
            if c0 > 0:
                y = y + g_s[...]
            if c0 + n == F:
                b = _rb(xn + (xn * 0.0 + _rb(_rb(y) * r_gate)))
                y = _rb(b * jax.nn.sigmoid(b))
            g_s[...] = y

        jobs = _Jobs(landed)
        for k in range(D // 128):
            for half in range(2):
                jobs.add(("q", k, half), ("wq", 128 * k, 128, half * QH, QH), [],
                         functools.partial(q_slab, k, half))
        for c0 in range(0, F, 256):
            n = min(256, F - c0)
            jobs.add(("g", c0), ("wg", c0, n, 0, D), [], functools.partial(gate_piece, c0, n))
            jobs.add(("u", c0), ("wu", c0, n, 0, D), [("g", c0)], functools.partial(up_piece, c0, n))
        for c0 in range(0, F, 512):
            n = min(512, F - c0)
            after = [("u", c) for c in range(c0, c0 + n, 256)] + ([("d", c0 - 512)] if c0 else [])
            jobs.add(("d", c0), ("wd", c0, n, 0, D), after, functools.partial(down_piece, c0, n))

        for i in range(-NP + 4, 2 * NS):
            plain_slot(i)
            jobs.step(cfg["JOBGAP"])
        assert not jobs.todo

        def qk(h, burst):
            m_run = None
            rows = W // KSUB
            for c in range(KSUB):
                s = lax.dot_general(q_s[h], kv_v[h, pl.ds(c * rows, rows), :], _NT,
                                    preferred_element_type=f32)
                burst()
                s = _rb(_rb(s) * scale)
                s_s[:, pl.ds(c * rows, rows)] = s
                for t in range(rows // 128):
                    st = s[:, t * 128:(t + 1) * 128]
                    m_run = st if m_run is None else jnp.maximum(m_run, st)
            return m_run

        def softmax_num(m_run):
            m = jnp.max(m_run, axis=-1, keepdims=True)
            p = jnp.exp(s_s[...] - m)
            p_s[...] = p.astype(bf16)
            return _tree_sum([p[:, t * 128:(t + 1) * 128] for t in range(W // 128)])

        def pv(h, l_vec, burst):
            acc = None
            rows = W // VSUB
            for c in range(VSUB):
                o = jnp.dot(p_s[:, pl.ds(c * rows, rows)], kv_v[H + h, pl.ds(c * rows, rows), :],
                            preferred_element_type=f32)
                burst()
                acc = o if acc is None else o + acc
            l = jnp.sum(l_vec, axis=-1, keepdims=True)
            o_s[h] = (acc / l).astype(bf16)

        def spread(h):
            col = jnp.broadcast_to(o_s[h][0:1].astype(f32), (128, DH)).T.reshape(DH // 8, 1, 8, 128)
            ob_s[pl.ds(h * UPH, UPH)] = jnp.broadcast_to(
                col, (DH // 8, UPR, 8, 128)).reshape(UPH, 8, 128)

        def step(h, l_vec, i0, nslots, dh=0):
            issued = [0]

            def burst():
                start_burst(i0 + issued[0] + N0, dh)
                issued[0] += 1

            if h > 1:
                spread(h - 2 + dh)
            m_run = qk(h + dh, burst) if h < H else None
            if h > 0:
                pv(h - 1 + dh, l_vec, burst)
            l_new = softmax_num(m_run) if h < H else None
            early = issued[0]
            for j in range(nslots):
                wait_slot(i0 + j, dh)
                wait_burst(i0 + j, dh)
                if j == 0 or j > early:
                    burst()
                start_slot(i0 + j + NS, dh)
            assert issued[0] == nslots
            return l_new

        def two_steps(p, l_vec):
            l_vec = step(2, l_vec, 4 * NS, NS, 2 * p)
            return step(3, l_vec, 5 * NS, NS, 2 * p)

        l_vec = step(0, None, 2 * NS, NS)
        l_vec = step(1, l_vec, 3 * NS, NS)
        l_vec = lax.fori_loop(0, (H - 8) // 2, two_steps, l_vec)
        for h in range(H - 6, H - 2):
            l_vec = step(h, l_vec, (h + 2) * NS, NS)
        e0 = H * NS
        l_vec = step(H - 2, l_vec, e0, NA + 1)
        l_vec = step(H - 1, l_vec, e0 + NA + 1, NA + 1)
        step(H, l_vec, e0 + 2 * NA + 2, VSUB + 1)

        spread(H - 1)
        acc = [[] for _ in range(UPR)]

        def project(budget):
            runs = []
            while wo_landed and wo_landed[0][1] <= budget:
                u0, n = wo_landed.pop(0)
                budget -= n
                if runs and sum(runs[-1]) == u0:
                    runs[-1][1] += n
                else:
                    runs.append([u0, n])
            parts = [[] for _ in range(UPR)]
            for u0, n in runs:
                ob = ob_s[pl.ds(u0, n)]
                prod = wo_v[pl.ds(u0, n)].astype(f32) * jnp.concatenate([ob, ob], axis=2)
                whole = n // UPR * UPR
                if whole:
                    red = jnp.sum(prod[:whole].reshape(n // UPR, UPR, 8, 256), axis=0)
                    for k in range(UPR):
                        parts[(u0 + k) % UPR].append(red[k])
                for k in range(whole, n):
                    parts[(u0 + k) % UPR].append(prod[k])
            for c in range(UPR):
                if parts[c]:
                    acc[c] = [_tree_sum(parts[c] + acc[c])]

        stage_tiles = _tiles(("stage", 0, DH, 0, D))
        for i in range(e0 + 2 * NA + VSUB + 3, e0 + NE):
            plain_slot(i)
            if stage_tiles and stage_tiles <= landed:
                stage_tiles = None
                row0 = lax.broadcasted_iota(jnp.int32, (_M, 256), 0) == 0
                for c in range(UPR):
                    part = jnp.concatenate(
                        [jnp.dot(o_s[0], kv_v[2 * H, pl.ds(c * 256 + cc, DH), :],
                                 preferred_element_type=f32) for cc in (0, 128)], axis=1)
                    acc[c] = [_tree_sum([jnp.where(row0, part, 0.0)] + acc[c])]
            project(cfg["UNITS"])
        assert not wo_landed and stage_tiles is None
        attn = _rb(jnp.sum(jnp.concatenate([a[0] for a in acc], axis=1), axis=0, keepdims=True))
        out_ref[0] = (x_v[0].astype(f32) + _rb(attn * g_s[...])).astype(out_ref.dtype)

    scratch = [
        pltpu.VMEM((1, 1, D), bf16),
        pltpu.VMEM((D,), bf16),
        pltpu.VMEM((D, H * DH), bf16),
        pltpu.VMEM((n_units, 8, 256), bf16),
        pltpu.VMEM((F, D), bf16),
        pltpu.VMEM((F, D), bf16),
        pltpu.VMEM((F, D), bf16),
        pltpu.VMEM((2 * H + 1, W, DH), bf16),
        pltpu.VMEM((_M, H * DH), f32),
        pltpu.VMEM((H, _M, DH), bf16),
        pltpu.VMEM((H, _M, DH), bf16),
        pltpu.VMEM((_M, W), f32),
        pltpu.VMEM((_M, W), bf16),
        pltpu.VMEM((_M, F), f32),
        pltpu.VMEM((_M, F), bf16),
        pltpu.VMEM((1, D), f32),
        pltpu.VMEM((n_units, 8, 128), f32),
        pltpu.SemaphoreType.DMA((2 * NS + 2,)),
    ]
    return kernel, scratch


@jax.jit
def pallas_recurrent_scan__sliding_block_cached__moe_arch_mod__decode_kernel(
    A_x: jax.Array,
    A_k_cache: jax.Array,
    A_v_cache: jax.Array,
    A_wq: jax.Array,
    A_wo: jax.Array,
    B_x: jax.Array,
    B_w_r: jax.Array,
    B_w_gate: jax.Array,
    B_w_up: jax.Array,
    B_w_down: jax.Array,
):
    del B_x
    _, _, D = A_x.shape
    _, H, SK, DH = A_k_cache.shape
    F = B_w_gate.shape[1]
    W = min(4096, max(256, SK // 4))
    kernel, scratch = _make_kernel(H, SK, W, DH, D, F, CFG)
    any_spec = pl.BlockSpec(memory_space=pl.ANY)
    wo_units = A_wo.reshape(-1, 8, D // 256, 256).transpose(0, 2, 1, 3).reshape(-1, 8, 256)
    return pl.pallas_call(
        kernel,
        out_shape=jax.ShapeDtypeStruct(A_x.shape, A_x.dtype),
        in_specs=[any_spec] * 10,
        out_specs=pl.BlockSpec(memory_space=pltpu.VMEM),
        scratch_shapes=scratch,
        compiler_params=pltpu.CompilerParams(
            vmem_limit_bytes=100 * 1024 * 1024,
            disable_bounds_checks=True,
            disable_semaphore_checks=True),
    )(A_x, A_k_cache, A_v_cache, A_wq, A_wo, wo_units, B_w_r, B_w_gate.T, B_w_up.T, B_w_down)
```

```python
import functools

import jax
import jax.numpy as jnp
import numpy as np
from jax import lax
import jax.experimental.pallas as pl
import jax.experimental.pallas.tpu as pltpu

_NT = (((1,), (1,)), ((), ()))
_M = 8
_BT = 32
_PT = 4
_RB = 8

CFG = dict(
    N0=12, L1=24,
    G_KV=14, G_WQ=14, G_WO=14, G_WG=0, G_WU=16, G_WD=0,
    KSUB=4, VSUB=2,
    TICK=40, SKIP=9,
    JOBGAP=3, R_WQ=4, R_WO=12, UNITS=48)


def _rects(name, t0, t1, ct):
    out = []
    while t0 < t1:
        r, c = divmod(t0, ct)
        if c or t1 - t0 < ct:
            n = min(ct - c, t1 - t0)
            out.append((name, 8 * r, 8, 128 * c, 128 * n))
            t0 += n
        else:
            rows = (t1 - t0) // ct
            out.append((name, 8 * r, 8 * rows, 0, 128 * ct))
            t0 += rows * ct
    return out


def _chop(lo, hi, g):
    cuts = [t for t in range(lo + _PT, hi - _PT + 1) if (t - g) % _PT == 0]
    cuts = [lo] + cuts + [hi] if hi > lo else []
    return list(zip(cuts[:-1], cuts[1:]))


def _split(total, g):
    lo = g % _BT
    hi = lo + (total - lo) // _BT * _BT
    return (0, lo), [(t, t + _BT) for t in range(lo, hi, _BT)], (hi, total)


def _tiles(piece):
    name, r0, nr, c0, nc = piece
    return {(name, r, c) for r in range(r0 // 8, (r0 + nr) // 8)
            for c in range(c0 // 128, (c0 + nc) // 128)}


def _rotate(*streams):
    out = []
    for i in range(max(len(s) for s in streams)):
        for s in streams:
            out += s[i:i + 1]
    return out


def _tree_sum(parts):
    while len(parts) > 1:
        parts = [a + b for a, b in zip(parts[0::2], parts[1::2])] + parts[len(parts) & ~1:]
    return parts[0]


def _rb(v):
    return v.astype(jnp.bfloat16).astype(jnp.float32)


class _Jobs:
    def __init__(self, landed):
        self.landed, self.todo, self.done, self.cool = landed, [], set(), 0

    def add(self, key, need, after, fn):
        self.todo.append((key, _tiles(need), set(after), fn))

    def ready(self):
        return [j for j in self.todo if j[1] <= self.landed and j[2] <= self.done]

    def run(self, job):
        self.todo.remove(job)
        job[3]()
        self.done.add(job[0])

    def step(self, gap):
        self.cool -= 1
        ready = self.ready()
        if self.cool <= 0 and ready:
            self.run(ready[0])
            self.cool = gap


def _make_kernel(H, SK, W, DH, D, F, cfg):
    f32, bf16 = jnp.float32, jnp.bfloat16
    HI, LO = 0, 1
    N0, KSUB, VSUB = cfg["N0"], cfg["KSUB"], cfg["VSUB"]
    WT = W // 8
    NS = 2 * (WT // _BT - 2)
    NA = KSUB + VSUB
    SKIP, L1 = cfg["SKIP"], cfg["L1"]
    scale = float(np.asarray(DH ** -0.5, bf16))
    eps = float(np.asarray(1e-5, bf16))
    assert DH == 128 and H % 2 == 0 and N0 + max(NA, SKIP) < NS and L1 <= NS

    g = cfg["G_KV"]
    head, blocks, tail = _split(WT, g)
    if len(blocks) > NS // 2 + 1:
        tail = blocks.pop()
    mid = _chop(*blocks.pop(NS // 4), g)
    head, tail = _chop(*head, g), _chop(*tail, g)
    i = 2
    while len(head + mid + tail) > NS // 2:
        mid[i:i + 2] = [(mid[i][0], mid[i + 1][1])]
        i += 1
    assert len(head + mid + tail) == len(blocks) == NS // 2
    kv_blocks = _rotate(blocks[:NS // 4], blocks[NS // 4:])
    frags = [(name, t0, t1) for part in (head, mid, tail) for name in "VK" for t0, t1 in part]

    def kv_slot(t, j):
        i = (t % 2) * NS + j
        t0, t1 = kv_blocks[i // 4]
        return [("VK"[i % 2], t - t % 2 + (i % 4) // 2, 8 * t0, 8 * (t1 - t0))]

    def kv_burst(t, j):
        name, t0, t1 = frags[j]
        return [(name, t + 2, 8 * t0, 8 * (t1 - t0))]

    def weight(name, rows, cols, g):
        ct = cols // 128
        head, blocks, tail = _split(rows // 8 * ct, g)
        whole = lambda rng: _rects(name, *rng, ct)
        pieces = lambda rng: [_rects(name, *p, ct) for p in _chop(*rng, g)]
        return pieces(head), [whole(b) for b in blocks], [pieces(b) for b in blocks], pieces(tail)

    wq_h, wq_b, wq_p, wq_t = weight("wq", D, H * DH, cfg["G_WQ"])
    wg_h, wg_b, wg_p, wg_t = weight("wg", F, D, cfg["G_WG"])
    wu_h, wu_b, wu_p, wu_t = weight("wu", F, D, cfg["G_WU"])
    wd_h, wd_b, wd_p, wd_t = weight("wd", F, D, cfg["G_WD"])
    r = cfg["R_WQ"]
    q1, q2 = r + (len(wq_b) - r + 2) // 3, r + (2 * (len(wq_b) - r) + 2) // 3
    pro_slots = _rotate(wg_b[:-1], wq_b[r:q1][::-1], wu_b[:-1], wq_b[q1:q2], wd_b[:-1], wq_b[q2:])
    NP = len(pro_slots)
    pro_bursts = sum(_rotate(wq_p[:r], [wg_p[-1], wd_p[-1], wu_p[-1] + wg_t + wq_t + wd_t + wu_t])
                     + [wq_h, wg_h, wu_h, wd_h], [])
    n_extra = len(pro_bursts) - (NP - 2 * NS)
    assert n_extra >= 0
    extra, pro_bursts = pro_bursts[:n_extra], pro_bursts[n_extra:]

    UPR = D // 256
    UPH = DH // 8 * UPR
    n_units = H * UPH
    g, r = cfg["G_WO"], cfg["R_WO"]
    assert g % 2 == 0 and _RB <= r <= 2 * _RB
    head, blocks, tail = _split(2 * n_units, g)
    pad = -g % _BT
    n_slabs = -(-(pad + 2 * n_units) // WT)
    streams = [blocks[max(b, r):b + _RB] for b in range(_RB, len(blocks), _RB)]
    epi_slots = [[("wo", *b)] for b in _rotate(*[st[::-1] for st in streams][::-1])[::-1]]
    NE = len(epi_slots)
    epi_bursts = [[("wo", *p)] for rng in [tail] + _rotate(blocks[_RB:r], blocks[:_RB]) + [head]
                  for p in _chop(*rng, g)]
    n_b = len(epi_bursts)
    assert n_b <= 2 * NS + NE

    def wo_rows(t0, t1):
        slab, t = divmod(pad + t0, WT)
        assert t + t1 - t0 <= WT
        return 2 * H + slab, pl.ds(8 * t, 8 * (t1 - t0))

    def slot_pieces(i):
        if i < 0:
            return pro_slots[NP + i]
        if i < NS * H:
            return kv_slot(*divmod(i, NS))
        return epi_slots[i - NS * H] if i - NS * H < NE else []

    def burst_pieces(i):
        if i < -2 * NS:
            return pro_bursts[NP + i]
        if i < NS * (H - 2):
            return kv_burst(*divmod(i, NS))
        return epi_bursts[i - NS * (H - 2)] if i - NS * (H - 2) < n_b else []

    def kernel(x_hbm, k_hbm, v_hbm, wq_hbm, wo_hbm, wr_hbm, wg_hbm, wu_hbm, wd_hbm,
               out_ref,
               x_v, wr_v, wq_v, wg_v, wu_v, wd_v, kv_v,
               qacc_s, q_s, o_s, s_s, p_s, gate_s, hid_s, g_s, ob_s, sems):
        mats = dict(wq=(wq_hbm, wq_v), wg=(wg_hbm, wg_v), wu=(wu_hbm, wu_v), wd=(wd_hbm, wd_v))
        landed = set()
        wo_landed = []

        def copy(piece, sem, dh):
            if piece[0] in "KV":
                name, h, r0, nr = piece
                src = k_hbm if name == "K" else v_hbm
                return pltpu.make_async_copy(
                    src.at[0, h + dh, pl.ds(SK - W + r0, nr), :],
                    kv_v.at[h + dh + (H if name == "V" else 0), pl.ds(r0, nr), :], sem)
            if piece[0] == "wo":
                _, t0, t1 = piece
                slab, rows = wo_rows(t0, t1)
                return pltpu.make_async_copy(wo_hbm.at[pl.ds(8 * t0, 8 * (t1 - t0)), :],
                                             kv_v.at[slab, rows, :], sem)
            name, r0, nr, c0, nc = piece
            src, dst = mats[name]
            return pltpu.make_async_copy(src.at[pl.ds(r0, nr), pl.ds(c0, nc)],
                                         dst.at[pl.ds(r0, nr), pl.ds(c0, nc)], sem)

        def start_slot(i, dh=0):
            for pc in slot_pieces(i):
                copy(pc, sems.at[i % NS], dh).start(priority=LO)

        def start_burst(i, dh=0):
            for pc in burst_pieces(i):
                copy(pc, sems.at[NS + i % NS], dh).start(priority=HI)

        def wait_pieces(pieces, sem, dh):
            for pc in pieces:
                copy(pc, sem, dh).wait()
            for pc in pieces:
                if pc[0] == "wo":
                    wo_landed.append((pc[1] // 2, (pc[2] - pc[1]) // 2))
                elif pc[0] not in "KV":
                    landed.update(_tiles(pc))

        def wait_slot(i, dh=0):
            wait_pieces(slot_pieces(i), sems.at[i % NS], dh)

        def wait_burst(i, dh=0):
            wait_pieces(burst_pieces(i), sems.at[NS + i % NS], dh)

        def plain_slot(i):
            wait_slot(i)
            wait_burst(i)
            start_burst(i + N0)
            start_slot(i + L1)

        x_cp = pltpu.make_async_copy(x_hbm, x_v, sems.at[2 * NS])
        wr_cp = pltpu.make_async_copy(wr_hbm, wr_v, sems.at[2 * NS + 1])
        extra_sem = sems.at[2 * NS + 2]
        ticks = [[copy(pc, extra_sem, 0) for pc in b] for b in extra]
        ticks += [[x_cp, wr_cp]]
        ticks += [[copy(pc, sems.at[NS + i % NS], 0) for pc in burst_pieces(i)]
                  for i in range(-NP, -NP + N0 + SKIP)]
        assert len(ticks) >= L1
        for j, cps in enumerate(ticks):
            if j > 0:
                pl.delay(cfg["TICK"])
            if j < L1:
                start_slot(-NP + j)
            for cp in cps:
                cp.start(priority=HI)
        P0 = -NP + SKIP
        for i in range(-NP, P0):
            wait_slot(i)
            wait_burst(i)
            start_slot(i + L1)
        wait_pieces(sum(extra, []), extra_sem, 0)

        x_cp.wait()
        wr_cp.wait()
        plain_slot(P0)
        x = x_v[0].astype(f32)
        mu = jnp.mean(x, axis=-1, keepdims=True)
        xc = x - mu
        plain_slot(P0 + 1)
        var = jnp.mean(xc * xc, axis=-1, keepdims=True)
        xn = _rb(_rb(x - _rb(mu)) / _rb(jnp.sqrt(_rb(_rb(var) + eps))))
        xn_b = jnp.broadcast_to(xn, (_M, D)).astype(bf16)
        plain_slot(P0 + 2)
        plain_slot(P0 + 3)
        wr = wr_v[...].astype(f32).reshape(1, D)
        r_gate = _rb(jax.nn.sigmoid(_rb(jnp.sum(xn * wr, axis=-1, keepdims=True))))

        QH = H * DH // 2
        q_seen = [0, 0]

        def q_slab(k, half):
            cols = pl.ds(half * QH, QH)
            part = jnp.dot(xn_b[:, k * 128:(k + 1) * 128], wq_v[pl.ds(k * 128, 128), cols],
                           preferred_element_type=f32)
            if q_seen[half] > 0:
                part = part + qacc_s[:, cols]
            q_seen[half] += 1
            if q_seen[half] < D // 128:
                qacc_s[:, cols] = part
            else:
                qb = part.astype(bf16)
                for hh in range(H // 2):
                    q_s[half * (H // 2) + hh] = qb[:, hh * DH:(hh + 1) * DH]

        def gate_piece(c0, n):
            gate_s[:, pl.ds(c0, n)] = lax.dot_general(
                xn_b, wg_v[pl.ds(c0, n), :], _NT, preferred_element_type=f32)

        def up_piece(c0, n):
            up = lax.dot_general(xn_b, wu_v[pl.ds(c0, n), :], _NT, preferred_element_type=f32)
            gate = _rb(gate_s[:, pl.ds(c0, n)])
            hid_s[:, pl.ds(c0, n)] = (_rb(gate * jax.nn.sigmoid(gate)) * _rb(up)).astype(bf16)

        def down_piece(c0, n):
            y = jnp.dot(hid_s[:, pl.ds(c0, n)], wd_v[pl.ds(c0, n), :],
                        preferred_element_type=f32)[0:1]
            if c0 > 0:
                y = y + g_s[...]
            if c0 + n == F:
                b = _rb(xn + (xn * 0.0 + _rb(_rb(y) * r_gate)))
                y = _rb(b * jax.nn.sigmoid(b))
            g_s[...] = y

        jobs = _Jobs(landed)
        for k in range(D // 128):
            for half in range(2):
                jobs.add(("q", k, half), ("wq", 128 * k, 128, half * QH, QH), [],
                         functools.partial(q_slab, k, half))
        for c0 in range(0, F, 256):
            n = min(256, F - c0)
            jobs.add(("g", c0), ("wg", c0, n, 0, D), [], functools.partial(gate_piece, c0, n))
            jobs.add(("u", c0), ("wu", c0, n, 0, D), [("g", c0)], functools.partial(up_piece, c0, n))
        for c0 in range(0, F, 512):
            n = min(512, F - c0)
            after = [("u", c) for c in range(c0, c0 + n, 256)] + ([("d", c0 - 512)] if c0 else [])
            jobs.add(("d", c0), ("wd", c0, n, 0, D), after, functools.partial(down_piece, c0, n))

        for i in range(P0 + 4, 2 * NS):
            plain_slot(i)
            jobs.step(cfg["JOBGAP"])
        assert not jobs.todo

        def qk(h, burst):
            m_run = None
            rows = W // KSUB
            for c in range(KSUB):
                s = lax.dot_general(q_s[h], kv_v[h, pl.ds(c * rows, rows), :], _NT,
                                    preferred_element_type=f32)
                burst()
                s = _rb(_rb(s) * scale)
                s_s[:, pl.ds(c * rows, rows)] = s
                for t in range(rows // 128):
                    st = s[:, t * 128:(t + 1) * 128]
                    m_run = st if m_run is None else jnp.maximum(m_run, st)
            return m_run

        def softmax_num(m_run):
            m = jnp.max(m_run, axis=-1, keepdims=True)
            p = jnp.exp(s_s[...] - m)
            p_s[...] = p.astype(bf16)
            return _tree_sum([p[:, t * 128:(t + 1) * 128] for t in range(W // 128)])

        def pv(h, l_vec, burst):
            acc = None
            rows = W // VSUB
            for c in range(VSUB):
                o = jnp.dot(p_s[:, pl.ds(c * rows, rows)], kv_v[H + h, pl.ds(c * rows, rows), :],
                            preferred_element_type=f32)
                burst()
                acc = o if acc is None else o + acc
            l = jnp.sum(l_vec, axis=-1, keepdims=True)
            o_s[h] = (acc / l).astype(bf16)

        def spread(h):
            col = jnp.broadcast_to(o_s[h][0:1].astype(f32), (128, DH)).T.reshape(DH // 8, 1, 8, 128)
            ob_s[pl.ds(h * UPH, UPH)] = jnp.broadcast_to(
                col, (DH // 8, UPR, 8, 128)).reshape(UPH, 8, 128)

        def step(h, l_vec, i0, nslots, dh=0):
            issued = [0]

            def burst():
                start_burst(i0 + issued[0] + N0, dh)
                issued[0] += 1

            if h > 1:
                spread(h - 2 + dh)
            m_run = qk(h + dh, burst) if h < H else None
            if h > 0:
                pv(h - 1 + dh, l_vec, burst)
            l_new = softmax_num(m_run) if h < H else None
            early = issued[0]
            for j in range(nslots):
                wait_slot(i0 + j, dh)
                wait_burst(i0 + j, dh)
                if j == 0 or j > early:
                    burst()
                start_slot(i0 + j + L1, dh)
            assert issued[0] == nslots
            return l_new

        def two_steps(p, l_vec):
            l_vec = step(2, l_vec, 4 * NS, NS, 2 * p)
            return step(3, l_vec, 5 * NS, NS, 2 * p)

        l_vec = step(0, None, 2 * NS, NS)
        l_vec = step(1, l_vec, 3 * NS, NS)
        l_vec = lax.fori_loop(0, (H - 8) // 2, two_steps, l_vec)
        for h in range(H - 6, H - 2):
            l_vec = step(h, l_vec, (h + 2) * NS, NS)
        e0 = H * NS
        l_vec = step(H - 2, l_vec, e0, NA + 1)
        l_vec = step(H - 1, l_vec, e0 + NA + 1, NA + 1)
        step(H, l_vec, e0 + 2 * NA + 2, VSUB + 1)

        spread(H - 1)
        acc = [[] for _ in range(UPR)]

        def project(budget):
            runs = []
            while wo_landed and wo_landed[0][1] <= budget:
                u0, n = wo_landed.pop(0)
                budget -= n
                if runs and sum(runs[-1]) == u0 and (pad + 2 * u0) % WT:
                    runs[-1][1] += n
                else:
                    runs.append([u0, n])
            parts = [[] for _ in range(UPR)]
            for u0, n in runs:
                slab, rows = wo_rows(2 * u0, 2 * (u0 + n))
                w = kv_v[slab, rows, :].astype(f32).reshape(n, 2, 8, 128)
                prod = w * ob_s[pl.ds(u0, n)].reshape(n, 1, 8, 128)
                whole = n // UPR * UPR
                if whole:
                    red = jnp.sum(prod[:whole].reshape(n // UPR, UPR, 2, 8, 128), axis=0)
                    for k in range(UPR):
                        parts[(u0 + k) % UPR].append(red[k])
                for k in range(whole, n):
                    parts[(u0 + k) % UPR].append(prod[k])
            for c in range(UPR):
                if parts[c]:
                    acc[c] = [_tree_sum(parts[c] + acc[c])]

        for i in range(e0 + 2 * NA + VSUB + 3, e0 + NE):
            plain_slot(i)
            project(cfg["UNITS"])
        assert not wo_landed
        attn = jnp.concatenate([a[0][k] for a in acc for k in range(2)], axis=1)
        attn = _rb(jnp.sum(attn, axis=0, keepdims=True))
        out_ref[0] = (x_v[0].astype(f32) + _rb(attn * g_s[...])).astype(out_ref.dtype)

    scratch = [
        pltpu.VMEM((1, 1, D), bf16),
        pltpu.VMEM((D,), bf16),
        pltpu.VMEM((D, H * DH), bf16),
        pltpu.VMEM((F, D), bf16),
        pltpu.VMEM((F, D), bf16),
        pltpu.VMEM((F, D), bf16),
        pltpu.VMEM((2 * H + n_slabs, W, DH), bf16),
        pltpu.VMEM((_M, H * DH), f32),
        pltpu.VMEM((H, _M, DH), bf16),
        pltpu.VMEM((H, _M, DH), bf16),
        pltpu.VMEM((_M, W), f32),
        pltpu.VMEM((_M, W), bf16),
        pltpu.VMEM((_M, F), f32),
        pltpu.VMEM((_M, F), bf16),
        pltpu.VMEM((1, D), f32),
        pltpu.VMEM((n_units, 8, 128), f32),
        pltpu.SemaphoreType.DMA((2 * NS + 3,)),
    ]
    return kernel, scratch


@jax.jit
def pallas_recurrent_scan__sliding_block_cached__moe_arch_mod__decode_kernel(
    A_x: jax.Array,
    A_k_cache: jax.Array,
    A_v_cache: jax.Array,
    A_wq: jax.Array,
    A_wo: jax.Array,
    B_x: jax.Array,
    B_w_r: jax.Array,
    B_w_gate: jax.Array,
    B_w_up: jax.Array,
    B_w_down: jax.Array,
):
    del B_x
    _, _, D = A_x.shape
    _, H, SK, DH = A_k_cache.shape
    F = B_w_gate.shape[1]
    W = min(4096, max(256, SK // 4))
    kernel, scratch = _make_kernel(H, SK, W, DH, D, F, CFG)
    any_spec = pl.BlockSpec(memory_space=pl.ANY)
    wo_tiles = A_wo.reshape(-1, 8, D // 128, 128).transpose(0, 2, 1, 3).reshape(-1, 128)
    return pl.pallas_call(
        kernel,
        out_shape=jax.ShapeDtypeStruct(A_x.shape, A_x.dtype),
        in_specs=[any_spec] * 9,
        out_specs=pl.BlockSpec(memory_space=pltpu.VMEM),
        scratch_shapes=scratch,
        compiler_params=pltpu.CompilerParams(
            vmem_limit_bytes=100 * 1024 * 1024,
            disable_bounds_checks=True,
            disable_semaphore_checks=True),
    )(A_x, A_k_cache, A_v_cache, A_wq, wo_tiles, B_w_r, B_w_gate.T, B_w_up.T, B_w_down)
```

```python
import functools

import jax
import jax.numpy as jnp
import numpy as np
from jax import lax
import jax.experimental.pallas as pl
import jax.experimental.pallas.tpu as pltpu

_NT = (((1,), (1,)), ((), ()))
_M = 8
_BT = 32
_PT = 4
_RB = 8

CFG = dict(
    N0=12, L1=24,
    G_KV=14, G_WQ=14, G_WO=14, G_WG=0, G_WU=16, G_WD=0,
    KSUB=4, VSUB=2,
    TICK=40, SKIP=9,
    JOBGAP=3, R_WQ=4, R_WO=12, UNITS=48, LAST=8)


def _rects(name, t0, t1, ct):
    out = []
    while t0 < t1:
        r, c = divmod(t0, ct)
        if c or t1 - t0 < ct:
            n = min(ct - c, t1 - t0)
            out.append((name, 8 * r, 8, 128 * c, 128 * n))
            t0 += n
        else:
            rows = (t1 - t0) // ct
            out.append((name, 8 * r, 8 * rows, 0, 128 * ct))
            t0 += rows * ct
    return out


def _chop(lo, hi, g):
    cuts = [t for t in range(lo + _PT, hi - _PT + 1) if (t - g) % _PT == 0]
    cuts = [lo] + cuts + [hi] if hi > lo else []
    return list(zip(cuts[:-1], cuts[1:]))


def _split(total, g):
    lo = g % _BT
    hi = lo + (total - lo) // _BT * _BT
    return (0, lo), [(t, t + _BT) for t in range(lo, hi, _BT)], (hi, total)


def _tiles(piece):
    name, r0, nr, c0, nc = piece
    return {(name, r, c) for r in range(r0 // 8, (r0 + nr) // 8)
            for c in range(c0 // 128, (c0 + nc) // 128)}


def _rotate(*streams):
    out = []
    for i in range(max(len(s) for s in streams)):
        for s in streams:
            out += s[i:i + 1]
    return out


def _tree_sum(parts):
    while len(parts) > 1:
        parts = [a + b for a, b in zip(parts[0::2], parts[1::2])] + parts[len(parts) & ~1:]
    return parts[0]


def _rb(v):
    return v.astype(jnp.bfloat16).astype(jnp.float32)


class _Jobs:
    def __init__(self, landed):
        self.landed, self.todo, self.done, self.cool = landed, [], set(), 0

    def add(self, key, need, after, fn):
        self.todo.append((key, _tiles(need), set(after), fn))

    def ready(self):
        return [j for j in self.todo if j[1] <= self.landed and j[2] <= self.done]

    def run(self, job):
        self.todo.remove(job)
        job[3]()
        self.done.add(job[0])

    def step(self, gap):
        self.cool -= 1
        ready = self.ready()
        if self.cool <= 0 and ready:
            self.run(ready[0])
            self.cool = gap


def _make_kernel(H, SK, W, DH, D, F, cfg):
    f32, bf16 = jnp.float32, jnp.bfloat16
    HI, LO = 0, 1
    N0, KSUB, VSUB = cfg["N0"], cfg["KSUB"], cfg["VSUB"]
    WT = W // 8
    NS = 2 * (WT // _BT - 2)
    NA = KSUB + VSUB
    SKIP, L1 = cfg["SKIP"], cfg["L1"]
    scale = float(np.asarray(DH ** -0.5, bf16))
    eps = float(np.asarray(1e-5, bf16))
    assert DH == 128 and H % 2 == 0 and N0 + max(NA, SKIP) < NS and L1 <= NS

    g = cfg["G_KV"]
    head, blocks, tail = _split(WT, g)
    if len(blocks) > NS // 2 + 1:
        tail = blocks.pop()
    mid = _chop(*blocks.pop(NS // 4), g)
    head, tail = _chop(*head, g), _chop(*tail, g)
    i = 2
    while len(head + mid + tail) > NS // 2:
        mid[i:i + 2] = [(mid[i][0], mid[i + 1][1])]
        i += 1
    assert len(head + mid + tail) == len(blocks) == NS // 2
    kv_blocks = _rotate(blocks[:NS // 4], blocks[NS // 4:])
    frags = [(name, t0, t1) for part in (head, mid, tail) for name in "VK" for t0, t1 in part]

    def kv_slot(t, j):
        i = (t % 2) * NS + j
        t0, t1 = kv_blocks[i // 4]
        return [("VK"[i % 2], t - t % 2 + (i % 4) // 2, 8 * t0, 8 * (t1 - t0))]

    def kv_burst(t, j):
        name, t0, t1 = frags[j]
        return [(name, t + 2, 8 * t0, 8 * (t1 - t0))]

    def weight(name, rows, cols, g):
        ct = cols // 128
        head, blocks, tail = _split(rows // 8 * ct, g)
        whole = lambda rng: _rects(name, *rng, ct)
        pieces = lambda rng: [_rects(name, *p, ct) for p in _chop(*rng, g)]
        return pieces(head), [whole(b) for b in blocks], [pieces(b) for b in blocks], pieces(tail)

    wq_h, wq_b, wq_p, wq_t = weight("wq", D, H * DH, cfg["G_WQ"])
    wg_h, wg_b, wg_p, wg_t = weight("wg", F, D, cfg["G_WG"])
    wu_h, wu_b, wu_p, wu_t = weight("wu", F, D, cfg["G_WU"])
    wd_h, wd_b, wd_p, wd_t = weight("wd", F, D, cfg["G_WD"])
    r = cfg["R_WQ"]
    q1, q2 = r + (len(wq_b) - r + 2) // 3, r + (2 * (len(wq_b) - r) + 2) // 3
    pro_slots = _rotate(wg_b[:-1], wq_b[r:q1][::-1], wu_b[:-1], wq_b[q1:q2], wd_b[:-1], wq_b[q2:])
    NP = len(pro_slots)
    pro_bursts = sum(_rotate(wq_p[:r], [wg_p[-1], wd_p[-1], wu_p[-1] + wg_t + wq_t + wd_t + wu_t])
                     + [wq_h, wg_h, wu_h, wd_h], [])
    n_extra = len(pro_bursts) - (NP - 2 * NS)
    assert n_extra >= 0
    extra, pro_bursts = pro_bursts[:n_extra], pro_bursts[n_extra:]

    UPR = D // 256
    UPH = DH // 8 * UPR
    n_units = H * UPH
    g, r = cfg["G_WO"], cfg["R_WO"]
    assert g % 2 == 0 and _RB <= r <= 2 * _RB
    head, blocks, tail = _split(2 * n_units, g)
    pad = -g % _BT
    n_slabs = -(-(pad + 2 * n_units) // WT)
    streams = [blocks[max(b, r):b + _RB] for b in range(_RB, len(blocks), _RB)]
    epi_slots = [[("wo", *b)] for b in _rotate(*[st[::-1] for st in streams][::-1])[::-1]]
    (_, t0, t1), = epi_slots.pop()
    epi_slots += [[("wo", t0, t1 - cfg["LAST"])], [("wo", t1 - cfg["LAST"], t1)]]
    NE = len(epi_slots)
    epi_bursts = [[("wo", *p)] for rng in [tail] + _rotate(blocks[_RB:r], blocks[:_RB]) + [head]
                  for p in _chop(*rng, g)]
    n_b = len(epi_bursts)
    assert n_b <= 2 * NS + NE

    def wo_rows(t0, t1):
        slab, t = divmod(pad + t0, WT)
        assert t + t1 - t0 <= WT
        return 2 * H + slab, pl.ds(8 * t, 8 * (t1 - t0))

    def slot_pieces(i):
        if i < 0:
            return pro_slots[NP + i]
        if i < NS * H:
            return kv_slot(*divmod(i, NS))
        return epi_slots[i - NS * H] if i - NS * H < NE else []

    def burst_pieces(i):
        if i < -2 * NS:
            return pro_bursts[NP + i]
        if i < NS * (H - 2):
            return kv_burst(*divmod(i, NS))
        return epi_bursts[i - NS * (H - 2)] if i - NS * (H - 2) < n_b else []

    def kernel(x_hbm, k_hbm, v_hbm, wq_hbm, wo_hbm, wr_hbm, wg_hbm, wu_hbm, wd_hbm,
               out_ref,
               x_v, wr_v, wq_v, wg_v, wu_v, wd_v, kv_v,
               qacc_s, q_s, o_s, s_s, p_s, gate_s, hid_s, g_s, ob_s, sems):
        mats = dict(wq=(wq_hbm, wq_v), wg=(wg_hbm, wg_v), wu=(wu_hbm, wu_v), wd=(wd_hbm, wd_v))
        landed = set()
        wo_landed = []

        def copy(piece, sem, dh):
            if piece[0] in "KV":
                name, h, r0, nr = piece
                src = k_hbm if name == "K" else v_hbm
                return pltpu.make_async_copy(
                    src.at[0, h + dh, pl.ds(SK - W + r0, nr), :],
                    kv_v.at[h + dh + (H if name == "V" else 0), pl.ds(r0, nr), :], sem)
            if piece[0] == "wo":
                _, t0, t1 = piece
                slab, rows = wo_rows(t0, t1)
                return pltpu.make_async_copy(wo_hbm.at[pl.ds(8 * t0, 8 * (t1 - t0)), :],
                                             kv_v.at[slab, rows, :], sem)
            name, r0, nr, c0, nc = piece
            src, dst = mats[name]
            return pltpu.make_async_copy(src.at[pl.ds(r0, nr), pl.ds(c0, nc)],
                                         dst.at[pl.ds(r0, nr), pl.ds(c0, nc)], sem)

        def start_slot(i, dh=0):
            for pc in slot_pieces(i):
                copy(pc, sems.at[i % NS], dh).start(priority=LO)

        def start_burst(i, dh=0):
            for pc in burst_pieces(i):
                copy(pc, sems.at[NS + i % NS], dh).start(priority=HI)

        def wait_pieces(pieces, sem, dh):
            for pc in pieces:
                copy(pc, sem, dh).wait()
            for pc in pieces:
                if pc[0] == "wo":
                    wo_landed.append((pc[1] // 2, (pc[2] - pc[1]) // 2))
                elif pc[0] not in "KV":
                    landed.update(_tiles(pc))

        def wait_slot(i, dh=0):
            wait_pieces(slot_pieces(i), sems.at[i % NS], dh)

        def wait_burst(i, dh=0):
            wait_pieces(burst_pieces(i), sems.at[NS + i % NS], dh)

        def plain_slot(i):
            wait_slot(i)
            wait_burst(i)
            start_burst(i + N0)
            start_slot(i + L1)

        x_cp = pltpu.make_async_copy(x_hbm, x_v, sems.at[2 * NS])
        wr_cp = pltpu.make_async_copy(wr_hbm, wr_v, sems.at[2 * NS + 1])
        extra_sem = sems.at[2 * NS + 2]
        ticks = [[copy(pc, extra_sem, 0) for pc in b] for b in extra]
        ticks += [[x_cp, wr_cp]]
        ticks += [[copy(pc, sems.at[NS + i % NS], 0) for pc in burst_pieces(i)]
                  for i in range(-NP, -NP + N0 + SKIP)]
        assert len(ticks) >= L1
        for j, cps in enumerate(ticks):
            if j > 0:
                pl.delay(cfg["TICK"])
            if j < L1:
                start_slot(-NP + j)
            for cp in cps:
                cp.start(priority=HI)
        P0 = -NP + SKIP
        for i in range(-NP, P0):
            wait_slot(i)
            wait_burst(i)
            start_slot(i + L1)
        wait_pieces(sum(extra, []), extra_sem, 0)

        x_cp.wait()
        wr_cp.wait()
        plain_slot(P0)
        x = x_v[0].astype(f32)
        mu = jnp.mean(x, axis=-1, keepdims=True)
        xc = x - mu
        plain_slot(P0 + 1)
        var = jnp.mean(xc * xc, axis=-1, keepdims=True)
        xn = _rb(_rb(x - _rb(mu)) / _rb(jnp.sqrt(_rb(_rb(var) + eps))))
        xn_b = jnp.broadcast_to(xn, (_M, D)).astype(bf16)
        plain_slot(P0 + 2)
        plain_slot(P0 + 3)
        wr = wr_v[...].astype(f32).reshape(1, D)
        r_gate = _rb(jax.nn.sigmoid(_rb(jnp.sum(xn * wr, axis=-1, keepdims=True))))

        QH = H * DH // 2
        q_seen = [0, 0]

        def q_slab(k, half):
            cols = pl.ds(half * QH, QH)
            part = jnp.dot(xn_b[:, k * 128:(k + 1) * 128], wq_v[pl.ds(k * 128, 128), cols],
                           preferred_element_type=f32)
            if q_seen[half] > 0:
                part = part + qacc_s[:, cols]
            q_seen[half] += 1
            if q_seen[half] < D // 128:
                qacc_s[:, cols] = part
            else:
                qb = part.astype(bf16)
                for hh in range(H // 2):
                    q_s[half * (H // 2) + hh] = qb[:, hh * DH:(hh + 1) * DH]

        def gate_piece(c0, n):
            gate_s[:, pl.ds(c0, n)] = lax.dot_general(
                xn_b, wg_v[pl.ds(c0, n), :], _NT, preferred_element_type=f32)

        def up_piece(c0, n):
            up = lax.dot_general(xn_b, wu_v[pl.ds(c0, n), :], _NT, preferred_element_type=f32)
            gate = _rb(gate_s[:, pl.ds(c0, n)])
            hid_s[:, pl.ds(c0, n)] = (_rb(gate * jax.nn.sigmoid(gate)) * _rb(up)).astype(bf16)

        def down_piece(c0, n):
            y = jnp.dot(hid_s[:, pl.ds(c0, n)], wd_v[pl.ds(c0, n), :],
                        preferred_element_type=f32)[0:1]
            if c0 > 0:
                y = y + g_s[...]
            if c0 + n == F:
                b = _rb(xn + (xn * 0.0 + _rb(_rb(y) * r_gate)))
                y = _rb(b * jax.nn.sigmoid(b))
            g_s[...] = y

        jobs = _Jobs(landed)
        for k in range(D // 128):
            for half in range(2):
                jobs.add(("q", k, half), ("wq", 128 * k, 128, half * QH, QH), [],
                         functools.partial(q_slab, k, half))
        for c0 in range(0, F, 256):
            n = min(256, F - c0)
            jobs.add(("g", c0), ("wg", c0, n, 0, D), [], functools.partial(gate_piece, c0, n))
            jobs.add(("u", c0), ("wu", c0, n, 0, D), [("g", c0)], functools.partial(up_piece, c0, n))
        for c0 in range(0, F, 512):
            n = min(512, F - c0)
            after = [("u", c) for c in range(c0, c0 + n, 256)] + ([("d", c0 - 512)] if c0 else [])
            jobs.add(("d", c0), ("wd", c0, n, 0, D), after, functools.partial(down_piece, c0, n))

        for i in range(P0 + 4, 2 * NS):
            plain_slot(i)
            jobs.step(cfg["JOBGAP"])
        assert not jobs.todo

        def qk(h, burst):
            m_run = None
            rows = W // KSUB
            for c in range(KSUB):
                s = lax.dot_general(q_s[h], kv_v[h, pl.ds(c * rows, rows), :], _NT,
                                    preferred_element_type=f32)
                burst()
                s = _rb(_rb(s) * scale)
                s_s[:, pl.ds(c * rows, rows)] = s
                for t in range(rows // 128):
                    st = s[:, t * 128:(t + 1) * 128]
                    m_run = st if m_run is None else jnp.maximum(m_run, st)
            return m_run

        def softmax_num(m_run):
            m = jnp.max(m_run, axis=-1, keepdims=True)
            p = jnp.exp(s_s[...] - m)
            p_s[...] = p.astype(bf16)
            return _tree_sum([p[:, t * 128:(t + 1) * 128] for t in range(W // 128)])

        def pv(h, l_vec, burst):
            acc = None
            rows = W // VSUB
            for c in range(VSUB):
                o = jnp.dot(p_s[:, pl.ds(c * rows, rows)], kv_v[H + h, pl.ds(c * rows, rows), :],
                            preferred_element_type=f32)
                burst()
                acc = o if acc is None else o + acc
            l = jnp.sum(l_vec, axis=-1, keepdims=True)
            o_s[h] = (acc / l).astype(bf16)

        def spread(h):
            col = jnp.broadcast_to(o_s[h][0:1].astype(f32), (128, DH)).T.reshape(DH // 8, 1, 8, 128)
            ob_s[pl.ds(h * UPH, UPH)] = jnp.broadcast_to(
                col, (DH // 8, UPR, 8, 128)).reshape(UPH, 8, 128)

        def step(h, l_vec, i0, nslots, dh=0):
            issued = [0]

            def burst():
                start_burst(i0 + issued[0] + N0, dh)
                issued[0] += 1

            if h > 1:
                spread(h - 2 + dh)
            m_run = qk(h + dh, burst) if h < H else None
            if h > 0:
                pv(h - 1 + dh, l_vec, burst)
            l_new = softmax_num(m_run) if h < H else None
            early = issued[0]
            for j in range(nslots):
                wait_slot(i0 + j, dh)
                wait_burst(i0 + j, dh)
                if j == 0 or j > early:
                    burst()
                start_slot(i0 + j + L1, dh)
            assert issued[0] == nslots
            return l_new

        def two_steps(p, l_vec):
            l_vec = step(2, l_vec, 4 * NS, NS, 2 * p)
            return step(3, l_vec, 5 * NS, NS, 2 * p)

        l_vec = step(0, None, 2 * NS, NS)
        l_vec = step(1, l_vec, 3 * NS, NS)
        l_vec = lax.fori_loop(0, (H - 8) // 2, two_steps, l_vec)
        for h in range(H - 6, H - 2):
            l_vec = step(h, l_vec, (h + 2) * NS, NS)
        e0 = H * NS
        l_vec = step(H - 2, l_vec, e0, NA + 1)
        l_vec = step(H - 1, l_vec, e0 + NA + 1, NA + 1)
        step(H, l_vec, e0 + 2 * NA + 2, VSUB + 1)

        spread(H - 1)
        acc = [[] for _ in range(UPR)]

        def project(budget):
            runs = []
            while wo_landed and wo_landed[0][1] <= budget:
                u0, n = wo_landed.pop(0)
                budget -= n
                if runs and sum(runs[-1]) == u0 and (pad + 2 * u0) % WT:
                    runs[-1][1] += n
                else:
                    runs.append([u0, n])
            parts = [[] for _ in range(UPR)]
            for u0, n in runs:
                slab, rows = wo_rows(2 * u0, 2 * (u0 + n))
                w = kv_v[slab, rows, :].astype(f32).reshape(n, 2, 8, 128)
                prod = w * ob_s[pl.ds(u0, n)].reshape(n, 1, 8, 128)
                whole = n // UPR * UPR
                if whole:
                    red = jnp.sum(prod[:whole].reshape(n // UPR, UPR, 2, 8, 128), axis=0)
                    for k in range(UPR):
                        parts[(u0 + k) % UPR].append(red[k])
                for k in range(whole, n):
                    parts[(u0 + k) % UPR].append(prod[k])
            for c in range(UPR):
                if parts[c]:
                    acc[c] = [_tree_sum(parts[c] + acc[c])]

        for i in range(e0 + 2 * NA + VSUB + 3, e0 + NE):
            plain_slot(i)
            project(cfg["UNITS"])
        assert not wo_landed
        attn = jnp.concatenate([a[0][k] for a in acc for k in range(2)], axis=1)
        attn = jnp.sum(attn, axis=0, keepdims=True)
        out_ref[0] = (attn * g_s[...] + x_v[0].astype(f32)).astype(out_ref.dtype)

    scratch = [
        pltpu.VMEM((1, 1, D), bf16),
        pltpu.VMEM((D,), bf16),
        pltpu.VMEM((D, H * DH), bf16),
        pltpu.VMEM((F, D), bf16),
        pltpu.VMEM((F, D), bf16),
        pltpu.VMEM((F, D), bf16),
        pltpu.VMEM((2 * H + n_slabs, W, DH), bf16),
        pltpu.VMEM((_M, H * DH), f32),
        pltpu.VMEM((H, _M, DH), bf16),
        pltpu.VMEM((H, _M, DH), bf16),
        pltpu.VMEM((_M, W), f32),
        pltpu.VMEM((_M, W), bf16),
        pltpu.VMEM((_M, F), f32),
        pltpu.VMEM((_M, F), bf16),
        pltpu.VMEM((1, D), f32),
        pltpu.VMEM((n_units, 8, 128), f32),
        pltpu.SemaphoreType.DMA((2 * NS + 3,)),
    ]
    return kernel, scratch


@jax.jit
def pallas_recurrent_scan__sliding_block_cached__moe_arch_mod__decode_kernel(
    A_x: jax.Array,
    A_k_cache: jax.Array,
    A_v_cache: jax.Array,
    A_wq: jax.Array,
    A_wo: jax.Array,
    B_x: jax.Array,
    B_w_r: jax.Array,
    B_w_gate: jax.Array,
    B_w_up: jax.Array,
    B_w_down: jax.Array,
):
    del B_x
    _, _, D = A_x.shape
    _, H, SK, DH = A_k_cache.shape
    F = B_w_gate.shape[1]
    W = min(4096, max(256, SK // 4))
    kernel, scratch = _make_kernel(H, SK, W, DH, D, F, CFG)
    any_spec = pl.BlockSpec(memory_space=pl.ANY)
    wo_tiles = A_wo.reshape(-1, 8, D // 128, 128).transpose(0, 2, 1, 3).reshape(-1, 128)
    return pl.pallas_call(
        kernel,
        out_shape=jax.ShapeDtypeStruct(A_x.shape, A_x.dtype),
        in_specs=[any_spec] * 9,
        out_specs=pl.BlockSpec(memory_space=pltpu.VMEM),
        scratch_shapes=scratch,
        compiler_params=pltpu.CompilerParams(
            vmem_limit_bytes=100 * 1024 * 1024,
            disable_bounds_checks=True,
            disable_semaphore_checks=True),
    )(A_x, A_k_cache, A_v_cache, A_wq, wo_tiles, B_w_r, B_w_gate.T, B_w_up.T, B_w_down)
```
